```python
import os as _os
_os.environ.setdefault("JAX_PLATFORMS", "cpu")
import jax
import jax.numpy as jnp

def _softmax(x, axis=-1):
    return jax.nn.softmax(x, axis=axis)
def _gelu(x):
    return jax.nn.gelu(x, approximate=True)
def _silu(x):
    return jax.nn.silu(x)
def _sigmoid(x):
    return jax.nn.sigmoid(x)
def _layernorm(x, axis=-1, eps=1e-5):
    m = jnp.mean(x, axis=axis, keepdims=True)
    v = jnp.var(x, axis=axis, keepdims=True)
    return (x - m) / jnp.sqrt(v + eps)
def _scatter_add(tgt, idx, src, axis=0):
    return tgt.at[idx].add(src)
def _segment_sum(src, seg, n):
    return jax.ops.segment_sum(src, seg, n)
class _Rng:
    def __init__(self, key):
        self._k = key
    def _next(self):
        self._k, sub = jax.random.split(self._k)
        return sub
    def normal(self, shape):
        return jax.random.normal(self._next(), shape, dtype=jnp.bfloat16)
    def randint(self, lo, hi, shape):
        return jax.random.randint(self._next(), shape, lo, hi, dtype=jnp.int32)
    def uniform(self, shape, lo=0.0, hi=1.0):
        return jax.random.uniform(self._next(), shape, jnp.bfloat16, lo, hi)
    def permutation(self, n):
        return jax.random.permutation(self._next(), n)


kernel_name = 'gated_mix__ssm_conv_s5__glu_gated_geglu__prompt'

def setup_inputs():
    _rng = _Rng(jax.random.key(int.from_bytes(__import__("os").urandom(4), "little")))
    _w = (lambda a: (lambda t: t.astype(jnp.bfloat16) if jnp.issubdtype(t.dtype, jnp.floating) else t)(jnp.asarray(a)))
    def _A_setup():
        B, S, D = 1, 2048, 1024
        P = D
        Lambda_re = -0.5 * jnp.exp((lambda *s: _rng.normal(s) * 0.4)(P))
        Lambda_im = (lambda *s: _rng.normal(s) * 0.4)(P) * 1.0
        B_re = (lambda *s: _rng.normal(s) * 0.4)(P, D) * (D ** -0.5)
        B_im = (lambda *s: _rng.normal(s) * 0.4)(P, D) * (D ** -0.5)
        C_re = (lambda *s: _rng.normal(s) * 0.4)(D, P) * (P ** -0.5)
        C_im = (lambda *s: _rng.normal(s) * 0.4)(D, P) * (P ** -0.5)
        log_dt = (lambda *s: _rng.normal(s) * 0.4)(P) * 0.3 - 2.0
        Dskip = (lambda *s: _rng.normal(s) * 0.4)(D)
        return {
            "x": _w((lambda *s: _rng.normal(s) * 0.05)(B, S, D)),
            "Lambda_re": _w(Lambda_re),
            "Lambda_im": _w(Lambda_im),
            "B_re": _w(B_re),
            "B_im": _w(B_im),
            "C_re": _w(C_re),
            "C_im": _w(C_im),
            "log_dt": _w(log_dt),
            "Dskip": _w(Dskip),
        }
    _A_in = _A_setup()

    def _B_setup():
        B, S, Dm, Df = 1, 2048, 1024, 3584
        return {
            "x": _w((lambda *s: _rng.normal(s) * 0.05)(B, S, Dm)),
            "w_gate": _w((lambda *s: _rng.normal(s) * 1.6)(Dm, Df) * (Dm ** -0.5)),
            "w_up": _w((lambda *s: _rng.normal(s) * 1.6)(Dm, Df) * (Dm ** -0.5)),
            "w_down": _w((lambda *s: _rng.normal(s) * 1.6)(Df, Dm) * (Df ** -0.5)),
        }
    _B_in = _B_setup()

    return {
        "A_x": _A_in["x"],
        "A_Lambda_re": _A_in["Lambda_re"],
        "A_Lambda_im": _A_in["Lambda_im"],
        "A_B_re": _A_in["B_re"],
        "A_B_im": _A_in["B_im"],
        "A_C_re": _A_in["C_re"],
        "A_C_im": _A_in["C_im"],
        "A_log_dt": _A_in["log_dt"],
        "A_Dskip": _A_in["Dskip"],
        "B_x": _B_in["x"],
        "B_w_gate": _B_in["w_gate"],
        "B_w_up": _B_in["w_up"],
        "B_w_down": _B_in["w_down"],
        "gate_w": _w((lambda *s: _rng.normal(s) * 0.05)(1024) * 16.0),
    }

def reference(A_x, A_Lambda_re, A_Lambda_im, A_B_re, A_B_im, A_C_re, A_C_im, A_log_dt, A_Dskip, B_x, B_w_gate, B_w_up, B_w_down, gate_w):
    def _A_ref(x, Lambda_re, Lambda_im, B_re, B_im, C_re, C_im, log_dt, Dskip):
        Bsz, L, H = x.shape
        Lam = Lambda_re + 1j * Lambda_im
        Bmat = B_re + 1j * B_im
        Cmat = C_re + 1j * C_im
        dt = jnp.exp(log_dt)
        Lam_bar = jnp.exp(dt * Lam)
        B_bar = ((Lam_bar - 1.0) / Lam)[:, None] * Bmat
        Bu = jnp.einsum("bld,pd->blp", x + 0j, B_bar)
        h = jnp.zeros_like(Bu[:, 0, :])
        hs = []
        for t in range(L):
            h = Lam_bar[None, :] * h + Bu[:, t, :]
            hs.append(h)
        hseq = jnp.stack(hs, 1)
        y = 2.0 * jnp.einsum("blp,dp->bld", hseq, Cmat).real + x * Dskip[None, None, :]
        return y

    def _B_ref(x, w_gate, w_up, w_down):
        g = jnp.einsum("bsd,df->bsf", x, w_gate)
        u = jnp.einsum("bsd,df->bsf", x, w_up)
        h = _gelu(g) * u
        return jnp.einsum("bsf,fd->bsd", h, w_down)

    x = A_x
    g = _sigmoid((x * gate_w).sum(-1, keepdims=True))
    a = _A_ref(x, A_Lambda_re, A_Lambda_im, A_B_re, A_B_im, A_C_re, A_C_im, A_log_dt, A_Dskip)
    b = _B_ref(x, B_w_gate, B_w_up, B_w_down)
    return g * a + (1 - g) * b
```

```python
import functools
import math

import numpy as np
import jax
import jax.numpy as jnp
from jax import lax
from jax.experimental import pallas as pl
from jax.experimental.pallas import tpu as pltpu

TM = 256
TA = 256
FC = 256
ILV = 1
F32 = jnp.float32
BF16 = jnp.bfloat16
NT = (((1,), (1,)), ((), ()))
K0 = math.sqrt(2.0 / math.pi)


def _cmul(ar, ai, br, bi):
    return ar * br - ai * bi, ar * bi + ai * br


def _kernel(x_hbm, lre_ref, lim_ref, ldt_ref, dsk_ref, gw_ref,
            bre_hbm, bim_hbm, cre_hbm, cim_hbm, wg_hbm, wu_hbm, wd_hbm,
            o_hbm,
            x_v, bre_v, bim_v, cre_v, cim_v, wg_v, wu_v, wd_v,
            ur_v, ui_v, h_v, hr_v, hi_v, o_v, coef_ref, carry_ref,
            xsem, wsem, osem, *, tm, ta, fc):
    S, D = x_v.shape
    P = bre_v.shape[0]
    DF = wg_v.shape[1]
    nA = S // ta
    nR = S // tm

    def x_copy(r):
        rows = pl.ds(r * ta, ta)
        return pltpu.make_async_copy(x_hbm.at[rows, :], x_v.at[rows, :], xsem.at[r])

    w_pairs = [(bre_hbm, bre_v), (bim_hbm, bim_v), (wg_hbm, wg_v), (wu_hbm, wu_v),
               (wd_hbm, wd_v), (cre_hbm, cre_v), (cim_hbm, cim_v)]
    w_copies = [pltpu.make_async_copy(s, d, wsem.at[i]) for i, (s, d) in enumerate(w_pairs)]

    x_copy(0).start()
    w_copies[0].start()
    w_copies[1].start()
    for r in range(1, nA):
        x_copy(r).start()
    for c in w_copies[2:]:
        c.start()

    dt = jnp.exp(ldt_ref[...].astype(F32)).astype(BF16).astype(F32)
    lre = lre_ref[...].astype(F32)
    lim = lim_ref[...].astype(F32)
    zr = dt * lre
    zi = dt * lim
    k = (lax.broadcasted_iota(jnp.int32, (8, P), 0) + 1).astype(F32)
    mag = jnp.exp(k * zr)
    pwr = mag * jnp.cos(k * zi)
    pwi = mag * jnp.sin(k * zi)
    coef_ref[0] = pwr
    coef_ref[1] = pwi
    ar = pwr[0:1] - 1.0
    ai = pwi[0:1]
    den = lre * lre + lim * lim
    coef_ref[2] = jnp.broadcast_to((ar * lre + ai * lim) / den, (8, P))
    coef_ref[3] = jnp.broadcast_to((ai * lre - ar * lim) / den, (8, P))
    row = lax.broadcasted_iota(jnp.int32, (8, P), 0)
    for n, s in enumerate((1, 2, 4)):
        coef_ref[4 + 2 * n] = jnp.where(row >= s, jnp.broadcast_to(pwr[s - 1:s], (8, P)), 0.0)
        coef_ref[5 + 2 * n] = jnp.where(row >= s, jnp.broadcast_to(pwi[s - 1:s], (8, P)), 0.0)
    carry_ref[...] = jnp.zeros_like(carry_ref)

    w_copies[0].wait()
    w_copies[1].wait()

    def phase_a(r, _):
        x_copy(r).wait()
        rows = pl.ds(pl.multiple_of(r * ta, ta), ta)
        x = x_v[rows, :]
        ur_v[rows, :] = lax.dot_general(x, bre_v[...], NT, preferred_element_type=F32)
        ui_v[rows, :] = lax.dot_general(x, bim_v[...], NT, preferred_element_type=F32)
        return 0

    lax.fori_loop(0, nA, phase_a, 0)
    for c in w_copies[2:]:
        c.wait()

    nchunk = DF // fc
    npiece = tm // 16

    def body(r, _):
        r0 = pl.multiple_of(r * tm, tm)
        rows = pl.ds(r0, tm)
        x = x_v[rows, :]
        xf = x.astype(F32)
        logit = jnp.sum(xf * gw_ref[...].astype(F32), axis=-1, keepdims=True)
        gate = jax.nn.sigmoid(logit)
        s1 = 1.0 - gate
        g2 = 2.0 * gate

        def scan_piece(q, HrHi):
            Hr, Hi = HrHi
            cr, ci = coef_ref[2], coef_ref[3]
            pwr, pwi = coef_ref[0], coef_ref[1]
            outs_r, outs_i = [], []
            for j in range(2):
                k8 = q * 16 + j * 8
                ur = ur_v[pl.ds(r0 + k8, 8), :]
                ui = ui_v[pl.ds(r0 + k8, 8), :]
                vr, vi = _cmul(cr, ci, ur, ui)
                for n, s in enumerate((1, 2, 4)):
                    mr, mi = coef_ref[4 + 2 * n], coef_ref[5 + 2 * n]
                    sr = pltpu.roll(vr, s, 0)
                    si = pltpu.roll(vi, s, 0)
                    vr, vi = vr + (mr * sr - mi * si), vi + (mr * si + mi * sr)
                hr = vr + (pwr * Hr - pwi * Hi)
                hi = vi + (pwr * Hi + pwi * Hr)
                Hr = jnp.broadcast_to(hr[7:8], (8, P))
                Hi = jnp.broadcast_to(hi[7:8], (8, P))
                gg = g2[k8:k8 + 8]
                outs_r.append(hr * gg)
                outs_i.append(hi * (-gg))
            hr_v[pl.ds(q * 16, 16), :] = jnp.concatenate(outs_r, axis=0).astype(BF16)
            hi_v[pl.ds(q * 16, 16), :] = jnp.concatenate(outs_i, axis=0).astype(BF16)
            return Hr, Hi

        H = (carry_ref[0], carry_ref[1])
        if not ILV:
            for q in range(npiece):
                H = scan_piece(q, H)
        q = 0
        for c in range(nchunk):
            cols = slice(c * fc, (c + 1) * fc)
            g = jnp.dot(x, wg_v[:, cols], preferred_element_type=F32)
            u = jnp.dot(x, wu_v[:, cols], preferred_element_type=F32)
            inner = g * (K0 + (K0 * 0.044715) * (g * g))
            hh = (0.5 * g) * (1.0 + jnp.tanh(inner)) * (u * s1)
            h_v[:, cols] = hh.astype(BF16)
            if ILV:
                qend = (c + 1) * npiece // nchunk
                while q < qend:
                    H = scan_piece(q, H)
                    q += 1
        carry_ref[0] = H[0]
        carry_ref[1] = H[1]
        acc = (gate * xf) * dsk_ref[...].astype(F32)
        acc = acc + jnp.dot(h_v[...], wd_v[...], preferred_element_type=F32)
        acc = acc + lax.dot_general(hr_v[...], cre_v[...], NT, preferred_element_type=F32)
        acc = acc + lax.dot_general(hi_v[...], cim_v[...], NT, preferred_element_type=F32)
        o_v[rows, :] = acc
        pltpu.make_async_copy(o_v.at[rows, :], o_hbm.at[rows, :], osem.at[r]).start()
        return 0

    lax.fori_loop(0, nR, body, 0)
    for r in range(nR):
        rows = pl.ds(r * tm, tm)
        pltpu.make_async_copy(o_v.at[rows, :], o_hbm.at[rows, :], osem.at[r]).wait()


@jax.jit
def pallas_gated_mix__ssm_conv_s5__glu_gated_geglu__prompt_kernel(
    A_x, A_Lambda_re, A_Lambda_im, A_B_re, A_B_im, A_C_re, A_C_im, A_log_dt, A_Dskip,
    B_x, B_w_gate, B_w_up, B_w_down, gate_w,
):
    Bsz, S, D = A_x.shape
    P = A_Lambda_re.shape[0]
    DF = B_w_gate.shape[1]
    tm, ta, fc = TM, TA, FC
    x2 = A_x.reshape(S, D)
    row = lambda a: a.reshape(1, -1)
    hbm = pl.BlockSpec(memory_space=pl.ANY)
    vmem = pl.BlockSpec(memory_space=pltpu.VMEM)
    out = pl.pallas_call(
        functools.partial(_kernel, tm=tm, ta=ta, fc=fc),
        in_specs=[hbm, vmem, vmem, vmem, vmem, vmem, hbm, hbm, hbm, hbm, hbm, hbm, hbm],
        out_specs=hbm,
        out_shape=jax.ShapeDtypeStruct((S, D), F32),
        scratch_shapes=[
            pltpu.VMEM((S, D), BF16),
            pltpu.VMEM((P, D), BF16), pltpu.VMEM((P, D), BF16),
            pltpu.VMEM((D, P), BF16), pltpu.VMEM((D, P), BF16),
            pltpu.VMEM((D, DF), BF16), pltpu.VMEM((D, DF), BF16), pltpu.VMEM((DF, D), BF16),
            pltpu.VMEM((S, P), F32), pltpu.VMEM((S, P), F32),
            pltpu.VMEM((tm, DF), BF16), pltpu.VMEM((tm, P), BF16), pltpu.VMEM((tm, P), BF16),
            pltpu.VMEM((S, D), F32),
            pltpu.VMEM((10, 8, P), F32), pltpu.VMEM((2, 8, P), F32),
            pltpu.SemaphoreType.DMA((S // ta,)), pltpu.SemaphoreType.DMA((7,)),
            pltpu.SemaphoreType.DMA((S // tm,)),
        ],
        compiler_params=pltpu.CompilerParams(vmem_limit_bytes=100 * 1024 * 1024),
    )(x2, row(A_Lambda_re), row(A_Lambda_im), row(A_log_dt), row(A_Dskip), row(gate_w),
      A_B_re, A_B_im, A_C_re, A_C_im, B_w_gate, B_w_up, B_w_down)
    return out.reshape(Bsz, S, D)
```

```python
import functools
import math
import numpy as np
import jax
import jax.numpy as jnp
from jax import lax
from jax.experimental import pallas as pl
from jax.experimental.pallas import tpu as pltpu

TM = 256
TA = 256
FC = 256
NCH = 1
PEEL = 1
BC = 256
SCOPES = 0
NOSCAN = 0
PRE = 1
GA = 0
NOGATE = 0
NS = 1
NSC = [512, 768, 896]
FLAGKW = {}
F32 = jnp.float32
BF16 = jnp.bfloat16
I32 = jnp.int32
NT = (((1,), (1,)), ((), ()))
K0 = math.sqrt(2.0 / math.pi)

import contextlib
def scope(name):
    return jax.named_scope(name) if SCOPES else contextlib.nullcontext()


def _cmul(ar, ai, br, bi):
    return ar * br - ai * bi, ar * bi + ai * br


def _row(v):
    return jnp.concatenate([v[j:j + 1, :] for j in range(v.shape[0])], axis=1)


def _kernel(x_hbm, lre_hbm, lim_hbm, ldt_hbm, dsk_hbm, gw_hbm,
            bre_hbm, bim_hbm, cre_hbm, cim_hbm, wg_hbm, wu_hbm, wd_hbm,
            o_hbm,
            x_v, b_v, cre_v, cim_v, wg_v, wu_v, wd_v,
            u_v, h_v, hr_v, hi_v, o_v, small_v, coef_ref, rows_ref, carry_ref, zero_ref, g_v,
            isem, osem, *, tm, ta, fc):
    S, D = x_v.shape
    P = b_v.shape[1]
    DF = wg_v.shape[1]
    nA = S // ta
    nR = S // tm
    nB = P // BC

    def x_copy(r):
        rows = pl.ds(r * ta, ta)
        return pltpu.make_async_copy(x_hbm.at[rows, :], x_v.at[rows, :], isem.at[r])

    b_copies = []
    for part, src in enumerate((bre_hbm, bim_hbm)):
        for i in range(nB):
            rows = pl.ds(i * BC, BC)
            b_copies.append(pltpu.make_async_copy(
                src.at[rows, :], b_v.at[part, rows, :], isem.at[nA + part * nB + i]))
    s_copies = [pltpu.make_async_copy(s, small_v.at[i], isem.at[nA + 2 * nB + i])
                for i, s in enumerate((lre_hbm, lim_hbm, ldt_hbm, dsk_hbm, gw_hbm))]
    w_pairs = [(wg_hbm, wg_v), (wu_hbm, wu_v), (wd_hbm, wd_v), (cre_hbm, cre_v), (cim_hbm, cim_v)]
    w_copies = [pltpu.make_async_copy(s, d, isem.at[nA + 2 * nB + 5 + i]) for i, (s, d) in enumerate(w_pairs)]

    with scope("issue"):
        for c in s_copies:
            c.start()
        x_copy(0).start()
        for c in b_copies:
            c.start()
        for r in range(1, nA):
            x_copy(r).start()
        for c in w_copies:
            c.start()

    with scope("coef"):
        for c in s_copies:
            c.wait()
        lre = _row(small_v[0].astype(F32))
        lim = _row(small_v[1].astype(F32))
        dt = jnp.exp(_row(small_v[2].astype(F32))).astype(BF16).astype(F32)
        rows_ref[0] = jnp.broadcast_to(_row(small_v[3].astype(F32)), (8, D))
        rows_ref[1] = jnp.broadcast_to(_row(small_v[4].astype(F32)), (8, D))
        zr = dt * lre
        zi = dt * lim
        sub = lax.broadcasted_iota(I32, (8, P), 0)
        k = jnp.where(sub == 0, 1, jnp.where(sub == 1, 2, 4)).astype(F32)
        mag = jnp.exp(k * zr)
        pwr = mag * jnp.cos(k * zi)
        pwi = mag * jnp.sin(k * zi)
        ar = pwr[0:1] - 1.0
        ai = pwi[0:1]
        den = lre * lre + lim * lim
        coef_ref[0] = jnp.broadcast_to(2.0 * (ar * lre + ai * lim) / den, (8, P))
        coef_ref[1] = jnp.broadcast_to(2.0 * (ai * lre - ar * lim) / den, (8, P))
        coef_ref[2] = jnp.where(sub == 0, jnp.broadcast_to(pwr[0:1], (8, P)), 0.0)
        coef_ref[3] = jnp.where(sub == 0, jnp.broadcast_to(pwi[0:1], (8, P)), 0.0)
        for n, s in enumerate((1, 2, 4)):
            coef_ref[4 + 2 * n] = jnp.where(sub >= s, jnp.broadcast_to(pwr[n:n + 1], (8, P)), 0.0)
            coef_ref[5 + 2 * n] = jnp.where(sub >= s, jnp.broadcast_to(pwi[n:n + 1], (8, P)), 0.0)
        carry_ref[...] = jnp.zeros_like(carry_ref)
        zero_ref[...] = jnp.zeros_like(zero_ref)

    def gate_of(x):
        logit = jnp.sum(x.astype(F32) * rows_ref[1, 0:1, :], axis=-1, keepdims=True)
        return jnp.broadcast_to(jax.nn.sigmoid(logit), (x.shape[0], 128))

    with scope("phaseA0"):
        if PEEL:
            x_copy(0).wait()
            x0 = x_v[0:ta, :]
            for part in range(2):
                for i in range(nB):
                    b_copies[part * nB + i].wait()
                    u_v[part, 0:ta, i * BC:(i + 1) * BC] = lax.dot_general(
                        x0, b_v[part, i * BC:(i + 1) * BC, :], NT, preferred_element_type=F32)
            if GA:
                g_v[0:ta, :] = gate_of(x0)
        else:
            for c in b_copies:
                c.wait()

    def phase_a(r, _):
        x_copy(r).wait()
        rows = pl.ds(pl.multiple_of(r * ta, ta), ta)
        x = x_v[rows, :]
        u_v[0, rows, :] = lax.dot_general(x, b_v[0], NT, preferred_element_type=F32)
        u_v[1, rows, :] = lax.dot_general(x, b_v[1], NT, preferred_element_type=F32)
        if GA:
            g_v[rows, :] = gate_of(x)
        return 0

    with scope("phaseA"):
        lax.fori_loop(1 if PEEL else 0, nA, phase_a, 0)
    with scope("waitW"):
        for c in w_copies:
            c.wait()

    nchunk = DF // fc
    LT = P // 128

    cuts = [0] + (NSC if NSC else [D * (n + 1) // NS for n in range(NS - 1)]) + [D]
    ncut = len(cuts) - 1

    def o_copy(r, n):
        rows = pl.ds(pl.multiple_of(r * tm, tm), tm)
        cols = pl.ds(cuts[n], cuts[n + 1] - cuts[n])
        return pltpu.make_async_copy(o_v.at[rows, cols], o_hbm.at[rows, cols], osem.at[r * ncut + n])

    def body(r, _):
        r0 = pl.multiple_of(r * tm, tm)
        rows = pl.ds(r0, tm)
        x = x_v[rows, :]
        xf = x.astype(F32)
        if NOGATE:
            gate = jnp.full((tm, 1), 0.5, F32)
            gb = jnp.broadcast_to(gate, (tm, 128))
        elif GA:
            gb = g_v[rows, :]
            gate = gb[:, 0:1]
        else:
            logit = jnp.sum(xf * rows_ref[1, 0:1, :], axis=-1, keepdims=True)
            gate = jax.nn.sigmoid(logit)
            gb = jnp.broadcast_to(gate, (tm, 128))
        ngb = -gb
        s1b = 1.0 - gb

        zero = zero_ref[...]
        prev = [None] * max(NCH, 1)
        for j in range(LT):
            ln = slice(j * 128, (j + 1) * 128)
            cr, ci = coef_ref[0, :, ln], coef_ref[1, :, ln]
            l0r, l0i = coef_ref[2, :, ln], coef_ref[3, :, ln]
            ms = [(coef_ref[4 + 2 * n, :, ln], coef_ref[5 + 2 * n, :, ln]) for n in range(3)]
            Hr, Hi = carry_ref[0, :, ln], carry_ref[1, :, ln]
            ch = j % max(NCH, 1)
            if NCH and prev[ch] is not None:
                Hr = pltpu.bitcast(pltpu.bitcast(Hr, I32) | (pltpu.bitcast(prev[ch], I32) & zero), F32)
            for q in range(tm // 16):
                outr, outi = [], []
                for t in range(2):
                    k8 = q * 16 + t * 8
                    ur = u_v[0, pl.ds(r0 + k8, 8), ln]
                    ui = u_v[1, pl.ds(r0 + k8, 8), ln]
                    if NOSCAN:
                        outr.append(ur)
                        outi.append(ui)
                        continue
                    vr, vi = _cmul(cr, ci, ur, ui)
                    vr, vi = vr + (l0r * Hr - l0i * Hi), vi + (l0r * Hi + l0i * Hr)
                    for s, (mr, mi) in zip((1, 2, 4), ms):
                        sr = pltpu.roll(vr, s, 0)
                        si = pltpu.roll(vi, s, 0)
                        vr, vi = vr + (mr * sr - mi * si), vi + (mr * si + mi * sr)
                    Hr = jnp.broadcast_to(vr[7:8], (8, 128))
                    Hi = jnp.broadcast_to(vi[7:8], (8, 128))
                    if PRE:
                        outr.append(vr * gb[k8:k8 + 8])
                        outi.append(vi * ngb[k8:k8 + 8])
                    else:
                        outr.append(vr)
                        outi.append(vi)
                hr_v[pl.ds(q * 16, 16), ln] = jnp.concatenate(outr, axis=0).astype(BF16)
                hi_v[pl.ds(q * 16, 16), ln] = jnp.concatenate(outi, axis=0).astype(BF16)
            carry_ref[0, :, ln] = Hr
            carry_ref[1, :, ln] = Hi
            prev[ch] = Hr

        for c in range(nchunk):
            cols = slice(c * fc, (c + 1) * fc)
            g = jnp.dot(x, wg_v[:, cols], preferred_element_type=F32)
            u = jnp.dot(x, wu_v[:, cols], preferred_element_type=F32)
            inner = g * (K0 + (K0 * 0.044715) * (g * g))
            hh = (g * (0.5 + 0.5 * jnp.tanh(inner))) * u
            if PRE:
                hh = hh * jnp.concatenate([s1b] * (fc // 128), axis=1)
            h_v[:, cols] = hh.astype(BF16)
        if PRE:
            acc = (xf * rows_ref[0, 0:1, :]) * jnp.concatenate([gb] * (D // 128), axis=1)
            acc = acc + jnp.dot(h_v[...], wd_v[...], preferred_element_type=F32)
            acc = acc + lax.dot_general(hr_v[...], cre_v[...], NT, preferred_element_type=F32)
            for n, (c0, c1) in enumerate(zip(cuts[:-1], cuts[1:])):
                o_v[rows, c0:c1] = acc[:, c0:c1] + lax.dot_general(
                    hi_v[...], cim_v[c0:c1, :], NT, preferred_element_type=F32)
                o_copy(r, n).start()
            return 0
        else:
            d1 = jnp.dot(h_v[...], wd_v[...], preferred_element_type=F32)
            y = lax.dot_general(hr_v[...], cre_v[...], NT, preferred_element_type=F32)
            y = y - lax.dot_general(hi_v[...], cim_v[...], NT, preferred_element_type=F32)
            y = y + xf * rows_ref[0, 0:1, :]
            o_v[rows, :] = d1 + jnp.concatenate([gb] * (D // 128), axis=1) * (y - d1)
        o_copy(r, 0).start()
        return 0

    with scope("main"):
        lax.fori_loop(0, nR, body, 0)
    with scope("tail"):
        for r in range(nR):
            for n in range(ncut):
                o_copy(r, n).wait()


@jax.jit
def pallas_gated_mix__ssm_conv_s5__glu_gated_geglu__prompt_kernel(
    A_x, A_Lambda_re, A_Lambda_im, A_B_re, A_B_im, A_C_re, A_C_im, A_log_dt, A_Dskip,
    B_x, B_w_gate, B_w_up, B_w_down, gate_w,
):
    Bsz, S, D = A_x.shape
    P = A_Lambda_re.shape[0]
    DF = B_w_gate.shape[1]
    tm, ta, fc = TM, TA, FC
    x2 = A_x.reshape(S, D)
    sq = lambda a: a.reshape(8, -1)
    hbm = pl.BlockSpec(memory_space=pl.ANY)
    out = pl.pallas_call(
        functools.partial(_kernel, tm=tm, ta=ta, fc=fc),
        in_specs=[hbm] * 13,
        out_specs=hbm,
        out_shape=jax.ShapeDtypeStruct((S, D), F32),
        scratch_shapes=[
            pltpu.VMEM((S, D), BF16),
            pltpu.VMEM((2, P, D), BF16),
            pltpu.VMEM((D, P), BF16), pltpu.VMEM((D, P), BF16),
            pltpu.VMEM((D, DF), BF16), pltpu.VMEM((D, DF), BF16), pltpu.VMEM((DF, D), BF16),
            pltpu.VMEM((2, S, P), F32),
            pltpu.VMEM((tm, DF), BF16), pltpu.VMEM((tm, P), BF16), pltpu.VMEM((tm, P), BF16),
            pltpu.VMEM((S, D), F32),
            pltpu.VMEM((5, 8, P // 8), BF16),
            pltpu.VMEM((10, 8, P), F32), pltpu.VMEM((2, 8, D), F32), pltpu.VMEM((2, 8, P), F32),
            pltpu.VMEM((8, 128), I32),
            pltpu.VMEM((S, 128), F32),
            pltpu.SemaphoreType.DMA((S // ta + 2 * (P // BC) + 10,)),
            pltpu.SemaphoreType.DMA((S // tm * (len(NSC) + 1 if NSC else NS),)),
        ],
        compiler_params=pltpu.CompilerParams(vmem_limit_bytes=100 * 1024 * 1024, **FLAGKW),
    )(x2, sq(A_Lambda_re), sq(A_Lambda_im), sq(A_log_dt), sq(A_Dskip), sq(gate_w),
      A_B_re, A_B_im, A_C_re, A_C_im, B_w_gate, B_w_up, B_w_down)
    return out.reshape(Bsz, S, D)
```

```python
import functools
import math
import numpy as np
import jax
import jax.numpy as jnp
from jax import lax
from jax.experimental import pallas as pl
from jax.experimental.pallas import tpu as pltpu

TM = 256
FC = 256
NCH = 1
BC = 256
BC2 = 128
ND = 512
NC = 128
TR = 64
TL = 128
UD = 2
UC = 2
EMB = 1
TRA = 16
NCK = 1
CHB = 0
DQ = 0
DR = 0
ORD = 1
EW = 1
SCOPES = 0
F32 = jnp.float32
BF16 = jnp.bfloat16
I32 = jnp.int32
U32 = jnp.uint32
NT = (((1,), (1,)), ((), ()))
K0 = math.sqrt(2.0 / math.pi)
ORDER = (2, 3, 0, 1, 4, 5, 6) if ORD else tuple(range(7))

import contextlib
def scope(name):
    return jax.named_scope(name) if SCOPES else contextlib.nullcontext()


def _bf(v):
    return pltpu.bitcast(v, BF16)


def _pk(v):
    return pltpu.bitcast(v.astype(BF16), U32)


def _cmul(ar, ai, br, bi):
    return ar * br - ai * bi, ar * bi + ai * br


def _row(v):
    return jnp.concatenate([v[j:j + 1, :] for j in range(v.shape[0])], axis=1)


def _halves(v):
    q = v.shape[0] // 16
    return (jnp.concatenate([v[16 * i:16 * i + 8] for i in range(q)], axis=0),
            jnp.concatenate([v[16 * i + 8:16 * i + 16] for i in range(q)], axis=0))


def _lsums(a11, a12, a21, a22):
    return [a11 + a22, a21 + a22, a11, a22, a11 + a12, a21 - a11, a12 - a22]


def _wsums(b11, b12, b21, b22):
    if EW:
        un = lambda v, k: pltpu.unpack_elementwise(v, index=k, packed_dtype=BF16, unpacked_dtype=F32)
        out = []
        parts = [[un(v, k) for v in (b11, b12, b21, b22)] for k in range(2)]
        sums = [(p[0] + p[3], p[1] - p[3], p[2] - p[0], p[0] + p[1], p[2] + p[3]) for p in parts]
        return [pltpu.pack_elementwise([lo, hi], packed_dtype=BF16) for lo, hi in zip(*sums)]
    b11, b12, b21, b22 = (_bf(v).astype(F32) for v in (b11, b12, b21, b22))
    return [_pk(v) for v in (b11 + b22, b12 - b22, b21 - b11, b11 + b12, b21 + b22)]


_SLOT = {0: 0, 2: 1, 3: 2, 5: 3, 6: 4}


def _products(dot):
    m = [None] * 7
    for i in ORDER:
        m[i] = dot(i)
    return (m[0] + m[3] - m[4] + m[6], m[2] + m[4], m[1] + m[3], m[0] - m[1] + m[2] + m[5])


def _kernel(x_hbm, lre_hbm, lim_hbm, ldt_hbm, dsk_hbm, gw_hbm,
            bre_hbm, bim_hbm, cre_hbm, cim_hbm, wg_hbm, wu_hbm, wd_hbm,
            o_hbm,
            x_v, b_v, cre_v, cim_v, wg_v, wu_v, wd_v, tgu_v, td_v, tc_v, tb_v,
            u_v, ld_v, lc_v, o_v, small_v, coef_ref, rows_ref, carry_ref, zero_ref,
            isem, osem):
    tm, fc = TM, FC
    S, D = 2 * x_v.shape[0], x_v.shape[1]
    P = b_v.shape[0]
    DF = wg_v.shape[1]
    nR = S // tm
    nB = P // BC
    HM, HD, HF = tm // 2, D // 2, DF // 2
    G = tm // 16

    def sh(ln, o):
        return slice(ln.start + o, ln.stop + o)

    def x_copy(r):
        rows = pl.ds(r * HM, HM)
        return pltpu.make_async_copy(x_hbm.bitcast(U32).at[rows, :], x_v.at[rows, :], isem.at[r])

    b_copies = {}
    for part, src in enumerate((bre_hbm, bim_hbm)):
        for i in range(nB):
            rows = pl.ds(i * BC // 2, BC // 2)
            b_copies[part, i] = pltpu.make_async_copy(
                src.bitcast(U32).at[rows, :], b_v.at[pl.ds(part * P // 2 + i * BC // 2, BC // 2), :], isem.at[nR + part * nB + i])
    s_copies = [pltpu.make_async_copy(s, small_v.at[i], isem.at[nR + 2 * nB + i])
                for i, s in enumerate((lre_hbm, lim_hbm, ldt_hbm, dsk_hbm, gw_hbm))]
    nS = nR - 1
    SW = DF // nS

    def gu_copy(which, sl):
        src, dst = ((wg_hbm, wg_v), (wu_hbm, wu_v))[which]
        cols = pl.ds(pl.multiple_of(sl * SW, SW), SW)
        return pltpu.make_async_copy(src.bitcast(U32).at[:, cols], dst.at[:, cols], isem.at[nR + 2 * nB + 10 + 2 * sl + which])

    w_pairs = [(wg_hbm, wg_v), (wu_hbm, wu_v), (wd_hbm, wd_v), (cre_hbm, cre_v), (cim_hbm, cim_v)]
    w_copies = [pltpu.make_async_copy(s.bitcast(U32), d, isem.at[nR + 2 * nB + 5 + i]) if (i >= 2 or not EMB) else None
                for i, (s, d) in enumerate(w_pairs)]

    with scope("issue"):
        for c in s_copies:
            c.start()
        x_copy(0).start()
        for part in range(2):
            for i in range(nB):
                b_copies[part, i].start()
        for r in range(1, nR):
            x_copy(r).start()
            if EMB:
                gu_copy(0, r - 1).start()
                gu_copy(1, r - 1).start()
        for c in w_copies[2 if EMB else 0:]:
            c.start()

    with scope("coef"):
        for c in s_copies:
            c.wait()
        lre = _row(small_v[0].astype(F32))
        lim = _row(small_v[1].astype(F32))
        dt = jnp.exp(_row(small_v[2].astype(F32))).astype(BF16).astype(F32)
        rows_ref[0] = jnp.broadcast_to(_row(small_v[3].astype(F32)), (8, D))
        rows_ref[1] = jnp.broadcast_to(_row(small_v[4].astype(F32)), (8, D))
        zr = dt * lre
        zi = dt * lim
        sub = lax.broadcasted_iota(I32, (8, P), 0)
        k = jnp.where(sub == 0, 1, jnp.where(sub == 1, 2, 4)).astype(F32)
        mag = jnp.exp(k * zr)
        pwr = mag * jnp.cos(k * zi)
        pwi = mag * jnp.sin(k * zi)
        ar = pwr[0:1] - 1.0
        ai = pwi[0:1]
        den = lre * lre + lim * lim
        coef_ref[0] = jnp.broadcast_to(2.0 * (ar * lre + ai * lim) / den, (8, P))
        coef_ref[1] = jnp.broadcast_to(2.0 * (ai * lre - ar * lim) / den, (8, P))
        coef_ref[2] = jnp.where(sub == 0, jnp.broadcast_to(pwr[0:1], (8, P)), 0.0)
        coef_ref[3] = jnp.where(sub == 0, jnp.broadcast_to(pwi[0:1], (8, P)), 0.0)
        for n, s in enumerate((1, 2, 4)):
            coef_ref[4 + 2 * n] = jnp.where(sub >= s, jnp.broadcast_to(pwr[n:n + 1], (8, P)), 0.0)
            coef_ref[5 + 2 * n] = jnp.where(sub >= s, jnp.broadcast_to(pwi[n:n + 1], (8, P)), 0.0)
        carry_ref[...] = jnp.zeros_like(carry_ref)
        zero_ref[...] = jnp.zeros_like(zero_ref)

    def tile_sums(get, put, ncols):
        for j in range(ncols // TL):
            ln = slice(j * TL, (j + 1) * TL)
            for n, v in enumerate(_wsums(*get(ln))):
                put(n, ln, v)

    def x_operands(xf):
        xt, xb = _halves(xf)
        return [v.astype(BF16) for v in _lsums(xt[:, 0:HD], xt[:, HD:D], xb[:, 0:HD], xb[:, HD:D])]

    def t_b(i, rws):
        if i == 1:
            return _bf(b_v[rws, 0:HD])
        if i == 4:
            return _bf(b_v[sh(rws, P // 2), HD:D])
        return _bf(tb_v[sh(rws, _SLOT[i] * P // 2), :])

    with scope("phaseA0"):
        x_copy(0).wait()
        x0 = _bf(x_v[0:HM, :])
        for part in range(2):
            for i in range(nB):
                b_copies[part, i].wait()
                rws = slice(i * BC // 2, (i + 1) * BC // 2)
                res = lax.dot_general(x0, _bf(b_v[sh(rws, part * P // 2), :]), NT, preferred_element_type=F32)
                u_v[part, 0:G, :, i * BC:(i + 1) * BC] = res.reshape(G, 16, BC)
                if part == 1 and not CHB:
                    for t in range(BC // TR):
                        rr = slice(rws.start + t * TR // 2, rws.start + (t + 1) * TR // 2)
                        tile_sums(lambda ln: (b_v[rr, ln], b_v[sh(rr, P // 2), ln], b_v[rr, sh(ln, HD)], b_v[sh(rr, P // 2), sh(ln, HD)]),
                                  lambda n, ln, v: tb_v.__setitem__((sh(rr, n * P // 2), ln), v), HD)
                if part == 1 and CHB:
                    zero = zero_ref[...]
                    dep = [None] * CHB
                    cnt = 0
                    for t in range(BC // 16):
                        rr = slice(rws.start + t * 8, rws.start + (t + 1) * 8)
                        for j in range(HD // 128):
                            ln = slice(j * 128, (j + 1) * 128)
                            ch = cnt % CHB
                            cnt += 1
                            b11, b22 = b_v[rr, ln], b_v[sh(rr, P // 2), sh(ln, HD)]
                            if dep[ch] is not None:
                                b11, b22 = b11 | dep[ch], b22 | dep[ch]
                            vs = _wsums(b11, b_v[sh(rr, P // 2), ln], b_v[rr, sh(ln, HD)], b22)
                            for k, v in enumerate(vs):
                                tb_v[sh(rr, k * P // 2), ln] = v
                            dep[ch] = pltpu.bitcast(pltpu.bitcast(vs[0], I32) & zero, U32)

    def phase_a(r, _):
        x_copy(r).wait()
        if EMB == 1:
            gu_copy(0, r - 1).wait()
            gu_copy(1, r - 1).wait()
        xf = _bf(x_v[pl.ds(pl.multiple_of(r * HM, HM), HM), :]).astype(F32)
        lx = x_operands(xf)
        g0 = pl.ds(pl.multiple_of(r * G, G), G)
        NG = P // BC2
        zero = zero_ref[...]
        c0 = pl.multiple_of((r - 1) * SW, SW)
        for n in range(NG):
            rws = slice(n * BC2 // 2, (n + 1) * BC2 // 2)
            cols = slice(n * BC2, (n + 1) * BC2)
            q4 = _products(lambda i: lax.dot_general(lx[i], t_b(i, rws), NT, preferred_element_type=F32))
            u_v[0, g0, 0:8, cols] = q4[0].reshape(G, 8, BC2)
            u_v[1, g0, 0:8, cols] = q4[1].reshape(G, 8, BC2)
            u_v[0, g0, 8:16, cols] = q4[2].reshape(G, 8, BC2)
            u_v[1, g0, 8:16, cols] = q4[3].reshape(G, 8, BC2)
            if EMB and n == 0:
                dep = [pltpu.bitcast(pltpu.bitcast(q4[0][0:8, 0:128], I32) & zero, U32)] * NCK
                cnt = 0
                for t in range(HD // TRA):
                    rr = slice(t * TRA // 2, (t + 1) * TRA // 2)
                    for j in range(SW // TL):
                        ln = pl.ds(c0 + j * TL, TL)
                        lo, hi = rr, sh(rr, HD // 2)
                        ch = cnt % NCK
                        cnt += 1
                        depr = jnp.concatenate([dep[ch]] * (TRA // 16), axis=0)
                        vs = _wsums(wg_v[lo, ln] | depr, wu_v[lo, ln], wg_v[hi, ln], wu_v[hi, ln] | depr)
                        for k, v in enumerate(vs):
                            tgu_v[sh(rr, k * HD // 2), ln] = v
                        dep[ch] = pltpu.bitcast(pltpu.bitcast(vs[0][0:8], I32) & zero, U32)
        return 0

    if EMB == 2:
        with scope("prewait"):
            for sl in range(nS):
                gu_copy(0, sl).wait()
                gu_copy(1, sl).wait()
    with scope("phaseA"):
        lax.fori_loop(1, nR, phase_a, 0)

    def transform(nrows, ncols, get, dst, unroll):
        slot = nrows // 2
        step = TR * unroll // 2

        def it(i, _):
            for t in range(unroll):
                base = pl.multiple_of(i * step + t * (TR // 2), TR // 2)
                rows = lambda o: pl.ds(base + o, TR // 2)
                tile_sums(functools.partial(get, rows), lambda n, ln, v: dst.__setitem__((rows(n * slot), ln), v), ncols)
            return 0
        lax.fori_loop(0, nrows // (2 * step), it, 0)

    with scope("xform_gu"):
      if not EMB:
        w_copies[0].wait()
        w_copies[1].wait()
        transform(HD, DF, lambda r, ln: (wg_v[r(0), ln], wu_v[r(0), ln], wg_v[r(HD // 2), ln], wu_v[r(HD // 2), ln]), tgu_v, 1)
    with scope("xform_d"):
        w_copies[2].wait()
        transform(HF, HD, lambda r, ln: (wd_v[r(0), ln], wd_v[r(0), sh(ln, HD)], wd_v[r(HF // 2), ln], wd_v[r(HF // 2), sh(ln, HD)]), td_v, UD)
    with scope("xform_c"):
        w_copies[3].wait()
        w_copies[4].wait()
        transform(HD, P, lambda r, ln: (cre_v[r(0), ln], cre_v[r(HD // 2), ln], cim_v[r(0), ln], cim_v[r(HD // 2), ln]), tc_v, UC)

    nchunk = DF // fc
    LT = P // 128
    ngrp = HD // NC

    def o_copy(r, n, half):
        g0 = pl.ds(pl.multiple_of(r * G, G), G)
        cols = pl.ds(half * HD + n * NC, NC)
        return pltpu.make_async_copy(o_v.at[g0, :, cols], o_hbm.at[g0, :, cols], osem.at[(r * ngrp + n) * 2 + half])

    def t_gu(i, cols):
        if i == 1:
            return _bf(wg_v[0:HD // 2, cols])
        if i == 4:
            return _bf(wu_v[HD // 2:HD, cols])
        return _bf(tgu_v[_SLOT[i] * HD // 2:(_SLOT[i] + 1) * HD // 2, cols])

    def t_d(i, cols):
        if i == 1:
            return _bf(wd_v[0:HF // 2, cols])
        if i == 4:
            return _bf(wd_v[HF // 2:HF, sh(cols, HD)])
        return _bf(td_v[_SLOT[i] * HF // 2:(_SLOT[i] + 1) * HF // 2, cols])

    def t_c(i, rws):
        if i == 1:
            return _bf(cre_v[rws, :])
        if i == 4:
            return _bf(cim_v[sh(rws, HD // 2), :])
        return _bf(tc_v[sh(rws, _SLOT[i] * HD // 2), :])

    def widen(v, n):
        return v if n == 128 else jnp.concatenate([v] * (n // 128), axis=1)

    def body(r, _):
        xf = _bf(x_v[pl.ds(pl.multiple_of(r * HM, HM), HM), :]).astype(F32)
        logit = jnp.sum(xf * rows_ref[1, 0:1, :], axis=-1, keepdims=True)
        gb = jnp.broadcast_to(jax.nn.sigmoid(logit), (tm, 128))
        ngb = -gb
        s1t, s1b = _halves(1.0 - gb)
        g0 = pl.multiple_of(r * G, G)

        zero = zero_ref[...]
        prev = None
        for j in range(LT):
            ln = slice(j * 128, (j + 1) * 128)
            cr, ci = coef_ref[0, :, ln], coef_ref[1, :, ln]
            l0r, l0i = coef_ref[2, :, ln], coef_ref[3, :, ln]
            ms = [(coef_ref[4 + 2 * n, :, ln], coef_ref[5 + 2 * n, :, ln]) for n in range(3)]
            Hr, Hi = carry_ref[0, :, ln], carry_ref[1, :, ln]
            if NCH and prev is not None:
                Hr = pltpu.bitcast(pltpu.bitcast(Hr, I32) | (pltpu.bitcast(prev, I32) & zero), F32)
            for z in range(tm // 32):
                outr, outi = [], []
                for t in range(4):
                    k = 4 * z + t
                    rws = slice((k % 2) * 8, (k % 2) * 8 + 8)
                    ur = u_v[0, g0 + k // 2, rws, ln]
                    ui = u_v[1, g0 + k // 2, rws, ln]
                    vr, vi = _cmul(cr, ci, ur, ui)
                    vr, vi = vr + (l0r * Hr - l0i * Hi), vi + (l0r * Hi + l0i * Hr)
                    for s, (mr, mi) in zip((1, 2, 4), ms):
                        sr = pltpu.roll(vr, s, 0)
                        si = pltpu.roll(vi, s, 0)
                        vr, vi = vr + (mr * sr - mi * si), vi + (mr * si + mi * sr)
                    Hr = jnp.broadcast_to(vr[7:8], (8, 128))
                    Hi = jnp.broadcast_to(vi[7:8], (8, 128))
                    outr.append(vr * gb[8 * k:8 * k + 8])
                    outi.append(vi * ngb[8 * k:8 * k + 8])
                cat = lambda v, a, b: jnp.concatenate([v[a], v[b]], axis=0)
                for i, v in enumerate(_lsums(cat(outr, 0, 2), cat(outi, 0, 2), cat(outr, 1, 3), cat(outi, 1, 3))):
                    lc_v[i * HM // 2 + 8 * z:i * HM // 2 + 8 * z + 8, ln] = _pk(v)
            carry_ref[0, :, ln] = Hr
            carry_ref[1, :, ln] = Hi
            prev = Hr

        def geglu(g, u, s):
            inner = g * (K0 + (K0 * 0.044715) * (g * g))
            return (g * (0.5 + 0.5 * jnp.tanh(inner))) * (u * s)

        lx = x_operands(xf)

        def hh_chunk(c):
            cols = slice(c * fc, (c + 1) * fc)
            gt, ut, gbo, ubo = _products(lambda i: jnp.dot(lx[i], t_gu(i, cols), preferred_element_type=F32))
            return geglu(gt, ut, widen(s1t, fc)), geglu(gbo, ubo, widen(s1b, fc))

        for c in range(nchunk // 2):
            t1, b1 = hh_chunk(c)
            t2, b2 = hh_chunk(c + nchunk // 2)
            for i, v in enumerate(_lsums(t1, t2, b1, b2)):
                ld_v[i * HM // 2:(i + 1) * HM // 2, c * fc:(c + 1) * fc] = _pk(v)

        bt, bb = _halves((xf * rows_ref[0, 0:1, :]) * widen(gb, D))
        parts = []
        for n in range(HD // ND):
            cols = slice(n * ND, (n + 1) * ND)
            parts.append(_products(lambda i: jnp.dot(_bf(ld_v[i * HM // 2:(i + 1) * HM // 2, :]), t_d(i, cols), preferred_element_type=F32)))
        joined = (lambda v: v[0]) if len(parts) == 1 else (lambda v: jnp.concatenate(v, axis=1))
        q4 = [joined([p[k] for p in parts]) for k in range(4)]
        acc = [bt[:, 0:HD] + q4[0], bt[:, HD:D] + q4[1], bb[:, 0:HD] + q4[2], bb[:, HD:D] + q4[3]]
        gs = pl.ds(g0, G)
        for n in range(ngrp):
            cols = slice(n * NC, (n + 1) * NC)
            cols2 = sh(cols, HD)
            rws = slice(n * NC // 2, (n + 1) * NC // 2)
            q4 = _products(lambda i: lax.dot_general(_bf(lc_v[i * HM // 2:(i + 1) * HM // 2, :]), t_c(i, rws), NT, preferred_element_type=F32))
            o_v[gs, 0:8, cols] = (acc[0][:, cols] + q4[0]).reshape(G, 8, NC)
            o_v[gs, 8:16, cols] = (acc[2][:, cols] + q4[2]).reshape(G, 8, NC)
            o_copy(r, n, 0).start()
            o_v[gs, 0:8, cols2] = (acc[1][:, cols] + q4[1]).reshape(G, 8, NC)
            o_v[gs, 8:16, cols2] = (acc[3][:, cols] + q4[3]).reshape(G, 8, NC)
            o_copy(r, n, 1).start()
        return 0

    with scope("main"):
        lax.fori_loop(0, nR, body, 0)
    with scope("tail"):
        for r in range(nR):
            for n in range(ngrp):
                for half in range(2):
                    o_copy(r, n, half).wait()


@jax.jit
def pallas_gated_mix__ssm_conv_s5__glu_gated_geglu__prompt_kernel(
    A_x, A_Lambda_re, A_Lambda_im, A_B_re, A_B_im, A_C_re, A_C_im, A_log_dt, A_Dskip,
    B_x, B_w_gate, B_w_up, B_w_down, gate_w,
):
    Bsz, S, D = A_x.shape
    P = A_Lambda_re.shape[0]
    DF = B_w_gate.shape[1]
    tm = TM
    x2 = A_x.reshape(S, D)
    sq = lambda a: a.reshape(8, -1)
    hbm = pl.BlockSpec(memory_space=pl.ANY)
    out = pl.pallas_call(
        _kernel,
        in_specs=[hbm] * 13,
        out_specs=hbm,
        out_shape=jax.ShapeDtypeStruct((S // 16, 16, D), F32),
        scratch_shapes=[
            pltpu.VMEM((S // 2, D), U32),
            pltpu.VMEM((P, D), U32),
            pltpu.VMEM((D // 2, P), U32), pltpu.VMEM((D // 2, P), U32),
            pltpu.VMEM((D // 2, DF), U32), pltpu.VMEM((D // 2, DF), U32), pltpu.VMEM((DF // 2, D), U32),
            pltpu.VMEM((5 * D // 4, DF), U32), pltpu.VMEM((5 * DF // 4, D // 2), U32),
            pltpu.VMEM((5 * D // 4, P), U32), pltpu.VMEM((5 * P // 2, D // 2), U32),
            pltpu.VMEM((2, S // 16, 16, P), F32),
            pltpu.VMEM((7 * tm // 4, DF // 2), U32), pltpu.VMEM((7 * tm // 4, P), U32),
            pltpu.VMEM((S // 16, 16, D), F32),
            pltpu.VMEM((5, 8, P // 8), BF16),
            pltpu.VMEM((10, 8, P), F32), pltpu.VMEM((2, 8, D), F32), pltpu.VMEM((2, 8, P), F32),
            pltpu.VMEM((8, 128), I32),
            pltpu.SemaphoreType.DMA((S // tm + 2 * (P // BC) + 10 + 2 * (S // tm),)),
            pltpu.SemaphoreType.DMA((S // tm * 2 * (D // 2 // NC),)),
        ],
        compiler_params=pltpu.CompilerParams(vmem_limit_bytes=120 * 1024 * 1024),
    )(x2, sq(A_Lambda_re), sq(A_Lambda_im), sq(A_log_dt), sq(A_Dskip), sq(gate_w),
      A_B_re, A_B_im, A_C_re, A_C_im, B_w_gate, B_w_up, B_w_down)
    return out.reshape(Bsz, S, D)
```

```python
import functools
import math

import numpy as np
import jax
import jax.numpy as jnp
from jax import lax
from jax.experimental import pallas as pl
from jax.experimental.pallas import tpu as pltpu

TM = 256
TA = 256
FC = 256
NCH = 1
PEEL = 1
BC = 256
SCOPES = 0
NOSCAN = 0
PRE = 1
GA = 0
NOGATE = 0
NS = 1
NSC = [512, 768, 896]

FLAGKW = {}
F32 = jnp.float32
BF16 = jnp.bfloat16
I32 = jnp.int32
NT = (((1,), (1,)), ((), ()))
K0 = math.sqrt(2.0 / math.pi)

import contextlib
def scope(name):
    return jax.named_scope(name) if SCOPES else contextlib.nullcontext()


def _cmul(ar, ai, br, bi):
    return ar * br - ai * bi, ar * bi + ai * br


def _row(v):
    return jnp.concatenate([v[j:j + 1, :] for j in range(v.shape[0])], axis=1)


def _kernel(x_hbm, lre_hbm, lim_hbm, ldt_hbm, dsk_hbm, gw_hbm,
            bre_hbm, bim_hbm, cre_hbm, cim_hbm, wg_hbm, wu_hbm, wd_hbm,
            o_hbm,
            x_v, b_v, cre_v, cim_v, wg_v, wu_v, wd_v,
            u_v, h_v, hr_v, hi_v, o_v, small_v, coef_ref, rows_ref, carry_ref, zero_ref, g_v,
            isem, osem, *, tm, ta, fc):
    S, D = x_v.shape
    P = b_v.shape[1]
    DF = wg_v.shape[1]
    nA = S // ta
    nR = S // tm
    nB = P // BC

    def x_copy(r):
        rows = pl.ds(r * ta, ta)
        return pltpu.make_async_copy(x_hbm.at[rows, :], x_v.at[rows, :], isem.at[r])

    b_copies = []
    for part, src in enumerate((bre_hbm, bim_hbm)):
        for i in range(nB):
            rows = pl.ds(i * BC, BC)
            b_copies.append(pltpu.make_async_copy(
                src.at[rows, :], b_v.at[part, rows, :], isem.at[nA + part * nB + i]))
    s_copies = [pltpu.make_async_copy(s, small_v.at[i], isem.at[nA + 2 * nB + i])
                for i, s in enumerate((lre_hbm, lim_hbm, ldt_hbm, dsk_hbm, gw_hbm))]
    w_pairs = [(wg_hbm, wg_v), (wu_hbm, wu_v), (wd_hbm, wd_v), (cre_hbm, cre_v), (cim_hbm, cim_v)]
    w_copies = [pltpu.make_async_copy(s, d, isem.at[nA + 2 * nB + 5 + i]) for i, (s, d) in enumerate(w_pairs)]

    with scope("issue"):
        for c in s_copies:
            c.start()
        x_copy(0).start()
        for c in b_copies:
            c.start()
        for r in range(1, nA):
            x_copy(r).start()
        for c in w_copies:
            c.start()

    with scope("coef"):
        for c in s_copies:
            c.wait()
        lre = _row(small_v[0].astype(F32))
        lim = _row(small_v[1].astype(F32))
        dt = jnp.exp(_row(small_v[2].astype(F32))).astype(BF16).astype(F32)
        rows_ref[0] = jnp.broadcast_to(_row(small_v[3].astype(F32)), (8, D))
        rows_ref[1] = jnp.broadcast_to(_row(small_v[4].astype(F32)), (8, D))
        zr = dt * lre
        zi = dt * lim
        sub = lax.broadcasted_iota(I32, (8, P), 0)
        k = jnp.where(sub == 0, 1, jnp.where(sub == 1, 2, 4)).astype(F32)
        mag = jnp.exp(k * zr)
        pwr = mag * jnp.cos(k * zi)
        pwi = mag * jnp.sin(k * zi)
        ar = pwr[0:1] - 1.0
        ai = pwi[0:1]
        den = lre * lre + lim * lim
        coef_ref[0] = jnp.broadcast_to(2.0 * (ar * lre + ai * lim) / den, (8, P))
        coef_ref[1] = jnp.broadcast_to(2.0 * (ai * lre - ar * lim) / den, (8, P))
        coef_ref[2] = jnp.where(sub == 0, jnp.broadcast_to(pwr[0:1], (8, P)), 0.0)
        coef_ref[3] = jnp.where(sub == 0, jnp.broadcast_to(pwi[0:1], (8, P)), 0.0)
        for n, s in enumerate((1, 2, 4)):
            coef_ref[4 + 2 * n] = jnp.where(sub >= s, jnp.broadcast_to(pwr[n:n + 1], (8, P)), 0.0)
            coef_ref[5 + 2 * n] = jnp.where(sub >= s, jnp.broadcast_to(pwi[n:n + 1], (8, P)), 0.0)
        carry_ref[...] = jnp.zeros_like(carry_ref)
        zero_ref[...] = jnp.zeros_like(zero_ref)

    def gate_of(x):
        logit = jnp.sum(x.astype(F32) * rows_ref[1, 0:1, :], axis=-1, keepdims=True)
        return jnp.broadcast_to(jax.nn.sigmoid(logit), (x.shape[0], 128))

    with scope("phaseA0"):
        if PEEL:
            x_copy(0).wait()
            x0 = x_v[0:ta, :]
            for part in range(2):
                for i in range(nB):
                    b_copies[part * nB + i].wait()
                    u_v[part, 0:ta, i * BC:(i + 1) * BC] = lax.dot_general(
                        x0, b_v[part, i * BC:(i + 1) * BC, :], NT, preferred_element_type=F32)
            if GA:
                g_v[0:ta, :] = gate_of(x0)
        else:
            for c in b_copies:
                c.wait()

    def phase_a(r, _):
        x_copy(r).wait()
        rows = pl.ds(pl.multiple_of(r * ta, ta), ta)
        x = x_v[rows, :]
        u_v[0, rows, :] = lax.dot_general(x, b_v[0], NT, preferred_element_type=F32)
        u_v[1, rows, :] = lax.dot_general(x, b_v[1], NT, preferred_element_type=F32)
        if GA:
            g_v[rows, :] = gate_of(x)
        return 0

    with scope("phaseA"):
        lax.fori_loop(1 if PEEL else 0, nA, phase_a, 0)
    with scope("waitW"):
        for c in w_copies:
            c.wait()

    nchunk = DF // fc
    LT = P // 128

    cuts = [0] + (NSC if NSC else [D * (n + 1) // NS for n in range(NS - 1)]) + [D]
    ncut = len(cuts) - 1

    def o_copy(r, n):
        rows = pl.ds(pl.multiple_of(r * tm, tm), tm)
        cols = pl.ds(cuts[n], cuts[n + 1] - cuts[n])
        return pltpu.make_async_copy(o_v.at[rows, cols], o_hbm.at[rows, cols], osem.at[r * ncut + n])

    def body(r, _):
        r0 = pl.multiple_of(r * tm, tm)
        rows = pl.ds(r0, tm)
        x = x_v[rows, :]
        xf = x.astype(F32)
        if NOGATE:
            gate = jnp.full((tm, 1), 0.5, F32)
            gb = jnp.broadcast_to(gate, (tm, 128))
        elif GA:
            gb = g_v[rows, :]
            gate = gb[:, 0:1]
        else:
            logit = jnp.sum(xf * rows_ref[1, 0:1, :], axis=-1, keepdims=True)
            gate = jax.nn.sigmoid(logit)
            gb = jnp.broadcast_to(gate, (tm, 128))
        ngb = -gb
        s1b = 1.0 - gb

        zero = zero_ref[...]
        prev = [None] * max(NCH, 1)
        for j in range(LT):
            ln = slice(j * 128, (j + 1) * 128)
            cr, ci = coef_ref[0, :, ln], coef_ref[1, :, ln]
            l0r, l0i = coef_ref[2, :, ln], coef_ref[3, :, ln]
            ms = [(coef_ref[4 + 2 * n, :, ln], coef_ref[5 + 2 * n, :, ln]) for n in range(3)]
            Hr, Hi = carry_ref[0, :, ln], carry_ref[1, :, ln]
            ch = j % max(NCH, 1)
            if NCH and prev[ch] is not None:
                Hr = pltpu.bitcast(pltpu.bitcast(Hr, I32) | (pltpu.bitcast(prev[ch], I32) & zero), F32)
            for q in range(tm // 16):
                outr, outi = [], []
                for t in range(2):
                    k8 = q * 16 + t * 8
                    ur = u_v[0, pl.ds(r0 + k8, 8), ln]
                    ui = u_v[1, pl.ds(r0 + k8, 8), ln]
                    if NOSCAN:
                        outr.append(ur)
                        outi.append(ui)
                        continue
                    vr, vi = _cmul(cr, ci, ur, ui)
                    vr, vi = vr + (l0r * Hr - l0i * Hi), vi + (l0r * Hi + l0i * Hr)
                    for s, (mr, mi) in zip((1, 2, 4), ms):
                        sr = pltpu.roll(vr, s, 0)
                        si = pltpu.roll(vi, s, 0)
                        vr, vi = vr + (mr * sr - mi * si), vi + (mr * si + mi * sr)
                    Hr = jnp.broadcast_to(vr[7:8], (8, 128))
                    Hi = jnp.broadcast_to(vi[7:8], (8, 128))
                    if PRE:
                        outr.append(vr * gb[k8:k8 + 8])
                        outi.append(vi * ngb[k8:k8 + 8])
                    else:
                        outr.append(vr)
                        outi.append(vi)
                hr_v[pl.ds(q * 16, 16), ln] = jnp.concatenate(outr, axis=0).astype(BF16)
                hi_v[pl.ds(q * 16, 16), ln] = jnp.concatenate(outi, axis=0).astype(BF16)
            carry_ref[0, :, ln] = Hr
            carry_ref[1, :, ln] = Hi
            prev[ch] = Hr

        for c in range(nchunk):
            cols = slice(c * fc, (c + 1) * fc)
            g = jnp.dot(x, wg_v[:, cols], preferred_element_type=F32)
            u = jnp.dot(x, wu_v[:, cols], preferred_element_type=F32)
            inner = g * (K0 + (K0 * 0.044715) * (g * g))
            hh = (g * (0.5 + 0.5 * jnp.tanh(inner))) * u
            if PRE:
                hh = hh * jnp.concatenate([s1b] * (fc // 128), axis=1)
            h_v[:, cols] = hh.astype(BF16)
        if PRE:
            acc = (xf * rows_ref[0, 0:1, :]) * jnp.concatenate([gb] * (D // 128), axis=1)
            acc = acc + jnp.dot(h_v[...], wd_v[...], preferred_element_type=F32)
            acc = acc + lax.dot_general(hr_v[...], cre_v[...], NT, preferred_element_type=F32)
            for n, (c0, c1) in enumerate(zip(cuts[:-1], cuts[1:])):
                o_v[rows, c0:c1] = acc[:, c0:c1] + lax.dot_general(
                    hi_v[...], cim_v[c0:c1, :], NT, preferred_element_type=F32)
                o_copy(r, n).start()
            return 0
        else:
            d1 = jnp.dot(h_v[...], wd_v[...], preferred_element_type=F32)
            y = lax.dot_general(hr_v[...], cre_v[...], NT, preferred_element_type=F32)
            y = y - lax.dot_general(hi_v[...], cim_v[...], NT, preferred_element_type=F32)
            y = y + xf * rows_ref[0, 0:1, :]
            o_v[rows, :] = d1 + jnp.concatenate([gb] * (D // 128), axis=1) * (y - d1)
        o_copy(r, 0).start()
        return 0

    with scope("main"):
        lax.fori_loop(0, nR, body, 0)
    with scope("tail"):
        for r in range(nR):
            for n in range(ncut):
                o_copy(r, n).wait()


@jax.jit
def pallas_gated_mix__ssm_conv_s5__glu_gated_geglu__prompt_kernel(
    A_x, A_Lambda_re, A_Lambda_im, A_B_re, A_B_im, A_C_re, A_C_im, A_log_dt, A_Dskip,
    B_x, B_w_gate, B_w_up, B_w_down, gate_w,
):
    Bsz, S, D = A_x.shape
    P = A_Lambda_re.shape[0]
    DF = B_w_gate.shape[1]
    tm, ta, fc = TM, TA, FC
    x2 = A_x.reshape(S, D)
    sq = lambda a: a.reshape(8, -1)
    hbm = pl.BlockSpec(memory_space=pl.ANY)
    out = pl.pallas_call(
        functools.partial(_kernel, tm=tm, ta=ta, fc=fc),
        in_specs=[hbm] * 13,
        out_specs=hbm,
        out_shape=jax.ShapeDtypeStruct((S, D), F32),
        scratch_shapes=[
            pltpu.VMEM((S, D), BF16),
            pltpu.VMEM((2, P, D), BF16),
            pltpu.VMEM((D, P), BF16), pltpu.VMEM((D, P), BF16),
            pltpu.VMEM((D, DF), BF16), pltpu.VMEM((D, DF), BF16), pltpu.VMEM((DF, D), BF16),
            pltpu.VMEM((2, S, P), F32),
            pltpu.VMEM((tm, DF), BF16), pltpu.VMEM((tm, P), BF16), pltpu.VMEM((tm, P), BF16),
            pltpu.VMEM((S, D), F32),
            pltpu.VMEM((5, 8, P // 8), BF16),
            pltpu.VMEM((10, 8, P), F32), pltpu.VMEM((2, 8, D), F32), pltpu.VMEM((2, 8, P), F32),
            pltpu.VMEM((8, 128), I32),
            pltpu.VMEM((S, 128), F32),
            pltpu.SemaphoreType.DMA((S // ta + 2 * (P // BC) + 10,)),
            pltpu.SemaphoreType.DMA((S // tm * (len(NSC) + 1 if NSC else NS),)),
        ],
        compiler_params=pltpu.CompilerParams(vmem_limit_bytes=100 * 1024 * 1024, **FLAGKW),
    )(x2, sq(A_Lambda_re), sq(A_Lambda_im), sq(A_log_dt), sq(A_Dskip), sq(gate_w),
      A_B_re, A_B_im, A_C_re, A_C_im, B_w_gate, B_w_up, B_w_down)
    return out.reshape(Bsz, S, D)
```

```python
import math

import jax
import jax.numpy as jnp
from jax import lax
from jax.experimental import pallas as pl
from jax.experimental.pallas import tpu as pltpu

TM = 256
FC = 256
BC = 256
CUTS = (512, 768, 896)

F32 = jnp.float32
BF16 = jnp.bfloat16
I32 = jnp.int32
U32 = jnp.uint32
NT = (((1,), (1,)), ((), ()))
K0 = math.sqrt(2.0 / math.pi)


def _bf(v):
    return pltpu.bitcast(v, BF16)


def _pk(v):
    return pltpu.bitcast(v.astype(BF16), U32)


def _cmul(ar, ai, br, bi):
    return ar * br - ai * bi, ar * bi + ai * br


def _row(v):
    return jnp.concatenate([v[j:j + 1, :] for j in range(v.shape[0])], axis=1)


def _widen(v, n):
    return v if n == 128 else jnp.concatenate([v] * (n // 128), axis=1)


def _kernel(x_hbm, lre_hbm, lim_hbm, ldt_hbm, dsk_hbm, gw_hbm,
            bre_hbm, bim_hbm, cre_hbm, cim_hbm, wg_hbm, wu_hbm, wd_hbm,
            o_hbm,
            x_v, b_v, cre_v, cim_v, wg_v, wu_v, wd_v,
            u_v, h_v, hr_v, hi_v, o_v, small_v, coef_ref, rows_ref, carry_ref, zero_ref,
            isem, osem):
    tm, fc = TM, FC
    S, D = 2 * x_v.shape[0], x_v.shape[1]
    P = b_v.shape[0]
    DF = wg_v.shape[1]
    nR = S // tm
    nB = P // BC
    hm = tm // 2

    def x_copy(r):
        rows = pl.ds(r * hm if isinstance(r, int) else pl.multiple_of(r * hm, hm), hm)
        return pltpu.make_async_copy(x_hbm.bitcast(U32).at[rows, :], x_v.at[rows, :], isem.at[r])

    b_copies = []
    for part, src in enumerate((bre_hbm, bim_hbm)):
        for i in range(nB):
            b_copies.append(pltpu.make_async_copy(
                src.bitcast(U32).at[pl.ds(i * BC // 2, BC // 2), :],
                b_v.at[pl.ds((part * P + i * BC) // 2, BC // 2), :],
                isem.at[nR + part * nB + i]))
    s_copies = [pltpu.make_async_copy(s, small_v.at[i], isem.at[nR + 2 * nB])
                for i, s in enumerate((lre_hbm, lim_hbm, ldt_hbm, dsk_hbm, gw_hbm))]
    w_copies = [pltpu.make_async_copy(s.bitcast(U32), d, isem.at[nR + 2 * nB + 1])
                for s, d in ((wg_hbm, wg_v), (wu_hbm, wu_v), (wd_hbm, wd_v),
                             (cre_hbm, cre_v), (cim_hbm, cim_v))]

    for c in s_copies:
        c.start()
    x_copy(0).start()
    for c in b_copies:
        c.start()
    for r in range(1, nR):
        x_copy(r).start()
    for c in w_copies:
        c.start()

    for c in s_copies:
        c.wait()
    lre = _row(small_v[0].astype(F32))
    lim = _row(small_v[1].astype(F32))
    dt = jnp.exp(_row(small_v[2].astype(F32))).astype(BF16).astype(F32)
    rows_ref[0] = jnp.broadcast_to(_row(small_v[3].astype(F32)), (8, D))
    rows_ref[1] = jnp.broadcast_to(_row(small_v[4].astype(F32)), (8, D))
    zr = dt * lre
    zi = dt * lim
    sub = lax.broadcasted_iota(I32, (8, P), 0)
    k = jnp.where(sub == 0, 1, jnp.where(sub == 1, 2, 4)).astype(F32)
    mag = jnp.exp(k * zr)
    pwr = mag * jnp.cos(k * zi)
    pwi = mag * jnp.sin(k * zi)
    ar = pwr[0:1] - 1.0
    ai = pwi[0:1]
    den = lre * lre + lim * lim
    coef_ref[0] = jnp.broadcast_to(2.0 * (ar * lre + ai * lim) / den, (8, P))
    coef_ref[1] = jnp.broadcast_to(2.0 * (ai * lre - ar * lim) / den, (8, P))
    coef_ref[2] = jnp.where(sub == 0, jnp.broadcast_to(pwr[0:1], (8, P)), 0.0)
    coef_ref[3] = jnp.where(sub == 0, jnp.broadcast_to(pwi[0:1], (8, P)), 0.0)
    for n, s in enumerate((1, 2, 4)):
        coef_ref[4 + 2 * n] = jnp.where(sub >= s, jnp.broadcast_to(pwr[n:n + 1], (8, P)), 0.0)
        coef_ref[5 + 2 * n] = jnp.where(sub >= s, jnp.broadcast_to(pwi[n:n + 1], (8, P)), 0.0)
    carry_ref[...] = jnp.zeros_like(carry_ref)
    zero_ref[...] = jnp.zeros_like(zero_ref)

    x_copy(0).wait()
    x0 = _bf(x_v[0:hm, :])
    for part in range(2):
        for i in range(nB):
            b_copies[part * nB + i].wait()
            rws = slice((part * P + i * BC) // 2, (part * P + (i + 1) * BC) // 2)
            u_v[part, 0:tm, i * BC:(i + 1) * BC] = lax.dot_general(
                x0, _bf(b_v[rws, :]), NT, preferred_element_type=F32)

    def phase_a(r, _):
        x_copy(r).wait()
        x = _bf(x_v[pl.ds(pl.multiple_of(r * hm, hm), hm), :])
        rows = pl.ds(pl.multiple_of(r * tm, tm), tm)
        u_v[0, rows, :] = lax.dot_general(x, _bf(b_v[0:P // 2, :]), NT, preferred_element_type=F32)
        u_v[1, rows, :] = lax.dot_general(x, _bf(b_v[P // 2:P, :]), NT, preferred_element_type=F32)
        return 0

    lax.fori_loop(1, nR, phase_a, 0)
    for c in w_copies:
        c.wait()

    cuts = [0, *CUTS, D]

    def o_copy(r, n):
        rows = pl.ds(r * tm if isinstance(r, int) else pl.multiple_of(r * tm, tm), tm)
        cols = pl.ds(cuts[n], cuts[n + 1] - cuts[n])
        return pltpu.make_async_copy(o_v.at[rows, cols], o_hbm.at[rows, cols], osem.at[0])

    def body(r, _):
        r0 = pl.multiple_of(r * tm, tm)
        rows = pl.ds(r0, tm)
        x = _bf(x_v[pl.ds(pl.multiple_of(r * hm, hm), hm), :])
        xf = x.astype(F32)
        logit = jnp.sum(xf * rows_ref[1, 0:1, :], axis=-1, keepdims=True)
        gate = jnp.broadcast_to(jax.nn.sigmoid(logit), (tm, 128))
        ngate = -gate
        rest = 1.0 - gate

        zero = zero_ref[...]
        prev = None
        for j in range(P // 128):
            ln = slice(j * 128, (j + 1) * 128)
            cr, ci = coef_ref[0, :, ln], coef_ref[1, :, ln]
            l0r, l0i = coef_ref[2, :, ln], coef_ref[3, :, ln]
            steps = [(coef_ref[4 + 2 * n, :, ln], coef_ref[5 + 2 * n, :, ln]) for n in range(3)]
            Hr, Hi = carry_ref[0, :, ln], carry_ref[1, :, ln]
            if prev is not None:
                Hr = pltpu.bitcast(pltpu.bitcast(Hr, I32) | (pltpu.bitcast(prev, I32) & zero), F32)
            for q in range(tm // 16):
                outr, outi = [], []
                for t in range(2):
                    k8 = q * 16 + t * 8
                    vr, vi = _cmul(cr, ci, u_v[0, pl.ds(r0 + k8, 8), ln], u_v[1, pl.ds(r0 + k8, 8), ln])
                    vr, vi = vr + (l0r * Hr - l0i * Hi), vi + (l0r * Hi + l0i * Hr)
                    for s, (mr, mi) in zip((1, 2, 4), steps):
                        sr = pltpu.roll(vr, s, 0)
                        si = pltpu.roll(vi, s, 0)
                        vr, vi = vr + (mr * sr - mi * si), vi + (mr * si + mi * sr)
                    Hr = jnp.broadcast_to(vr[7:8], (8, 128))
                    Hi = jnp.broadcast_to(vi[7:8], (8, 128))
                    outr.append(vr * gate[k8:k8 + 8])
                    outi.append(vi * ngate[k8:k8 + 8])
                hr_v[q * 8:q * 8 + 8, ln] = _pk(jnp.concatenate(outr, axis=0))
                hi_v[q * 8:q * 8 + 8, ln] = _pk(jnp.concatenate(outi, axis=0))
            carry_ref[0, :, ln] = Hr
            carry_ref[1, :, ln] = Hi
            prev = Hr

        for c in range(DF // fc):
            cols = slice(c * fc, (c + 1) * fc)
            g = jnp.dot(x, _bf(wg_v[:, cols]), preferred_element_type=F32)
            u = jnp.dot(x, _bf(wu_v[:, cols]), preferred_element_type=F32)
            inner = g * (K0 + (K0 * 0.044715) * (g * g))
            h_v[:, cols] = _pk((g * (0.5 + 0.5 * jnp.tanh(inner))) * (u * _widen(rest, fc)))

        acc = (xf * rows_ref[0, 0:1, :]) * _widen(gate, D)
        acc = acc + jnp.dot(_bf(h_v[...]), _bf(wd_v[...]), preferred_element_type=F32)
        acc = acc + lax.dot_general(_bf(hr_v[...]), _bf(cre_v[...]), NT, preferred_element_type=F32)
        for n, (c0, c1) in enumerate(zip(cuts[:-1], cuts[1:])):
            o_v[rows, c0:c1] = acc[:, c0:c1] + lax.dot_general(
                _bf(hi_v[...]), _bf(cim_v[c0 // 2:c1 // 2, :]), NT, preferred_element_type=F32)
            o_copy(r, n).start()
        return 0

    lax.fori_loop(0, nR, body, 0)
    for r in range(nR):
        for n in range(len(cuts) - 1):
            o_copy(r, n).wait()


@jax.jit
def pallas_gated_mix__ssm_conv_s5__glu_gated_geglu__prompt_kernel(
    A_x: jax.Array,
    A_Lambda_re: jax.Array,
    A_Lambda_im: jax.Array,
    A_B_re: jax.Array,
    A_B_im: jax.Array,
    A_C_re: jax.Array,
    A_C_im: jax.Array,
    A_log_dt: jax.Array,
    A_Dskip: jax.Array,
    B_x: jax.Array,
    B_w_gate: jax.Array,
    B_w_up: jax.Array,
    B_w_down: jax.Array,
    gate_w: jax.Array,
):
    del B_x
    Bsz, S, D = A_x.shape
    P = A_Lambda_re.shape[0]
    DF = B_w_gate.shape[1]
    rows = Bsz * S
    vec = lambda a: a.reshape(8, -1)
    hbm = pl.BlockSpec(memory_space=pl.ANY)
    out = pl.pallas_call(
        _kernel,
        in_specs=[hbm] * 13,
        out_specs=hbm,
        out_shape=jax.ShapeDtypeStruct((rows, D), F32),
        scratch_shapes=[
            pltpu.VMEM((rows // 2, D), U32),
            pltpu.VMEM((P, D), U32),
            pltpu.VMEM((D // 2, P), U32),
            pltpu.VMEM((D // 2, P), U32),
            pltpu.VMEM((D // 2, DF), U32),
            pltpu.VMEM((D // 2, DF), U32),
            pltpu.VMEM((DF // 2, D), U32),
            pltpu.VMEM((2, rows, P), F32),
            pltpu.VMEM((TM // 2, DF), U32),
            pltpu.VMEM((TM // 2, P), U32),
            pltpu.VMEM((TM // 2, P), U32),
            pltpu.VMEM((rows, D), F32),
            pltpu.VMEM((5, 8, P // 8), BF16),
            pltpu.VMEM((10, 8, P), F32),
            pltpu.VMEM((2, 8, D), F32),
            pltpu.VMEM((2, 8, P), F32),
            pltpu.VMEM((8, 128), I32),
            pltpu.SemaphoreType.DMA((rows // TM + 2 * (P // BC) + 2,)),
            pltpu.SemaphoreType.DMA((1,)),
        ],
        compiler_params=pltpu.CompilerParams(vmem_limit_bytes=100 * 1024 * 1024),
    )(A_x.reshape(rows, D), vec(A_Lambda_re), vec(A_Lambda_im), vec(A_log_dt), vec(A_Dskip),
      vec(gate_w), A_B_re, A_B_im, A_C_re, A_C_im, B_w_gate, B_w_up, B_w_down)
    return out.reshape(Bsz, S, D)
```

```python
import math

import jax
import jax.numpy as jnp
from jax import lax
from jax.experimental import pallas as pl
from jax.experimental.pallas import tpu as pltpu

TM = 256
FC = 256
BC = 256
CUTS = (512, 768, 896)

F32 = jnp.float32
BF16 = jnp.bfloat16
I32 = jnp.int32
NT = (((1,), (1,)), ((), ()))
K0 = math.sqrt(2.0 / math.pi)


def _cmul(ar, ai, br, bi):
    return ar * br - ai * bi, ar * bi + ai * br


def _row(v):
    return jnp.concatenate([v[j:j + 1, :] for j in range(v.shape[0])], axis=1)


def _widen(v, n):
    return v if n == 128 else jnp.concatenate([v] * (n // 128), axis=1)


def _kernel(x_hbm, lre_hbm, lim_hbm, ldt_hbm, dsk_hbm, gw_hbm,
            bre_hbm, bim_hbm, cre_hbm, cim_hbm, wg_hbm, wu_hbm, wd_hbm,
            o_hbm,
            x_v, b_v, cre_v, cim_v, wg_v, wu_v, wd_v,
            u_v, h_v, hr_v, hi_v, o_v, small_v, coef_ref, rows_ref, carry_ref, zero_ref,
            isem, osem):
    tm, fc = TM, FC
    S, D = x_v.shape
    P = b_v.shape[1]
    DF = wg_v.shape[1]
    nR = S // tm
    nB = P // BC

    def x_copy(r):
        rows = pl.ds(r * tm if isinstance(r, int) else pl.multiple_of(r * tm, tm), tm)
        return pltpu.make_async_copy(x_hbm.at[rows, :], x_v.at[rows, :], isem.at[r])

    b_copies = []
    for part, src in enumerate((bre_hbm, bim_hbm)):
        for i in range(nB):
            rows = pl.ds(i * BC, BC)
            b_copies.append(pltpu.make_async_copy(
                src.at[rows, :], b_v.at[part, rows, :], isem.at[nR + part * nB + i]))
    s_copies = [pltpu.make_async_copy(s, small_v.at[i], isem.at[nR + 2 * nB])
                for i, s in enumerate((lre_hbm, lim_hbm, ldt_hbm, dsk_hbm, gw_hbm))]
    w_copies = [pltpu.make_async_copy(s, d, isem.at[nR + 2 * nB + 1])
                for s, d in ((wg_hbm, wg_v), (wu_hbm, wu_v), (wd_hbm, wd_v),
                             (cre_hbm, cre_v), (cim_hbm, cim_v))]

    for c in s_copies:
        c.start()
    x_copy(0).start()
    for c in b_copies:
        c.start()
    for r in range(1, nR):
        x_copy(r).start()
    for c in w_copies:
        c.start()

    for c in s_copies:
        c.wait()
    lre = _row(small_v[0].astype(F32))
    lim = _row(small_v[1].astype(F32))
    dt = jnp.exp(_row(small_v[2].astype(F32))).astype(BF16).astype(F32)
    rows_ref[0] = jnp.broadcast_to(_row(small_v[3].astype(F32)), (8, D))
    rows_ref[1] = jnp.broadcast_to(_row(small_v[4].astype(F32)), (8, D))
    zr = dt * lre
    zi = dt * lim
    sub = lax.broadcasted_iota(I32, (8, P), 0)
    k = jnp.where(sub == 0, 1, jnp.where(sub == 1, 2, 4)).astype(F32)
    mag = jnp.exp(k * zr)
    pwr = mag * jnp.cos(k * zi)
    pwi = mag * jnp.sin(k * zi)
    ar = pwr[0:1] - 1.0
    ai = pwi[0:1]
    den = lre * lre + lim * lim
    coef_ref[0] = jnp.broadcast_to(2.0 * (ar * lre + ai * lim) / den, (8, P))
    coef_ref[1] = jnp.broadcast_to(2.0 * (ai * lre - ar * lim) / den, (8, P))
    coef_ref[2] = jnp.where(sub == 0, jnp.broadcast_to(pwr[0:1], (8, P)), 0.0)
    coef_ref[3] = jnp.where(sub == 0, jnp.broadcast_to(pwi[0:1], (8, P)), 0.0)
    for n, s in enumerate((1, 2, 4)):
        coef_ref[4 + 2 * n] = jnp.where(sub >= s, jnp.broadcast_to(pwr[n:n + 1], (8, P)), 0.0)
        coef_ref[5 + 2 * n] = jnp.where(sub >= s, jnp.broadcast_to(pwi[n:n + 1], (8, P)), 0.0)
    carry_ref[...] = jnp.zeros_like(carry_ref)
    zero_ref[...] = jnp.zeros_like(zero_ref)

    x_copy(0).wait()
    x0 = x_v[0:tm, :]
    for part in range(2):
        for i in range(nB):
            b_copies[part * nB + i].wait()
            u_v[part, 0:tm, i * BC:(i + 1) * BC] = lax.dot_general(
                x0, b_v[part, i * BC:(i + 1) * BC, :], NT, preferred_element_type=F32)

    def phase_a(r, _):
        x_copy(r).wait()
        rows = pl.ds(pl.multiple_of(r * tm, tm), tm)
        x = x_v[rows, :]
        u_v[0, rows, :] = lax.dot_general(x, b_v[0], NT, preferred_element_type=F32)
        u_v[1, rows, :] = lax.dot_general(x, b_v[1], NT, preferred_element_type=F32)
        return 0

    lax.fori_loop(1, nR, phase_a, 0)
    for c in w_copies:
        c.wait()

    cuts = [0, *CUTS, D]

    def o_copy(r, n):
        rows = pl.ds(r * tm if isinstance(r, int) else pl.multiple_of(r * tm, tm), tm)
        cols = pl.ds(cuts[n], cuts[n + 1] - cuts[n])
        return pltpu.make_async_copy(o_v.at[rows, cols], o_hbm.at[rows, cols], osem.at[0])

    def body(r, _):
        r0 = pl.multiple_of(r * tm, tm)
        rows = pl.ds(r0, tm)
        x = x_v[rows, :]
        xf = x.astype(F32)
        logit = jnp.sum(xf * rows_ref[1, 0:1, :], axis=-1, keepdims=True)
        gate = jnp.broadcast_to(jax.nn.sigmoid(logit), (tm, 128))
        ngate = -gate
        rest = 1.0 - gate

        zero = zero_ref[...]
        prev = None
        for j in range(P // 128):
            ln = slice(j * 128, (j + 1) * 128)
            cr, ci = coef_ref[0, :, ln], coef_ref[1, :, ln]
            l0r, l0i = coef_ref[2, :, ln], coef_ref[3, :, ln]
            steps = [(coef_ref[4 + 2 * n, :, ln], coef_ref[5 + 2 * n, :, ln]) for n in range(3)]
            Hr, Hi = carry_ref[0, :, ln], carry_ref[1, :, ln]
            if prev is not None:
                Hr = pltpu.bitcast(pltpu.bitcast(Hr, I32) | (pltpu.bitcast(prev, I32) & zero), F32)
            for q in range(tm // 16):
                outr, outi = [], []
                for t in range(2):
                    k8 = q * 16 + t * 8
                    vr, vi = _cmul(cr, ci, u_v[0, pl.ds(r0 + k8, 8), ln], u_v[1, pl.ds(r0 + k8, 8), ln])
                    vr, vi = vr + (l0r * Hr - l0i * Hi), vi + (l0r * Hi + l0i * Hr)
                    for s, (mr, mi) in zip((1, 2, 4), steps):
                        sr = pltpu.roll(vr, s, 0)
                        si = pltpu.roll(vi, s, 0)
                        vr, vi = vr + (mr * sr - mi * si), vi + (mr * si + mi * sr)
                    Hr = jnp.broadcast_to(vr[7:8], (8, 128))
                    Hi = jnp.broadcast_to(vi[7:8], (8, 128))
                    outr.append(vr * gate[k8:k8 + 8])
                    outi.append(vi * ngate[k8:k8 + 8])
                hr_v[q * 16:q * 16 + 16, ln] = jnp.concatenate(outr, axis=0).astype(BF16)
                hi_v[q * 16:q * 16 + 16, ln] = jnp.concatenate(outi, axis=0).astype(BF16)
            carry_ref[0, :, ln] = Hr
            carry_ref[1, :, ln] = Hi
            prev = Hr

        for c in range(DF // fc):
            cols = slice(c * fc, (c + 1) * fc)
            g = jnp.dot(x, wg_v[:, cols], preferred_element_type=F32)
            u = jnp.dot(x, wu_v[:, cols], preferred_element_type=F32)
            inner = g * (K0 + (K0 * 0.044715) * (g * g))
            h_v[:, cols] = ((g * (0.5 + 0.5 * jnp.tanh(inner))) * (u * _widen(rest, fc))).astype(BF16)

        acc = (xf * rows_ref[0, 0:1, :]) * _widen(gate, D)
        acc = acc + jnp.dot(h_v[...], wd_v[...], preferred_element_type=F32)
        acc = acc + lax.dot_general(hr_v[...], cre_v[...], NT, preferred_element_type=F32)
        for n, (c0, c1) in enumerate(zip(cuts[:-1], cuts[1:])):
            o_v[rows, c0:c1] = acc[:, c0:c1] + lax.dot_general(
                hi_v[...], cim_v[c0:c1, :], NT, preferred_element_type=F32)
            o_copy(r, n).start()
        return 0

    lax.fori_loop(0, nR, body, 0)
    for r in range(nR):
        for n in range(len(cuts) - 1):
            o_copy(r, n).wait()


@jax.jit
def pallas_gated_mix__ssm_conv_s5__glu_gated_geglu__prompt_kernel(
    A_x: jax.Array,
    A_Lambda_re: jax.Array,
    A_Lambda_im: jax.Array,
    A_B_re: jax.Array,
    A_B_im: jax.Array,
    A_C_re: jax.Array,
    A_C_im: jax.Array,
    A_log_dt: jax.Array,
    A_Dskip: jax.Array,
    B_x: jax.Array,
    B_w_gate: jax.Array,
    B_w_up: jax.Array,
    B_w_down: jax.Array,
    gate_w: jax.Array,
):
    del B_x
    Bsz, S, D = A_x.shape
    P = A_Lambda_re.shape[0]
    DF = B_w_gate.shape[1]
    rows = Bsz * S
    vec = lambda a: a.reshape(8, -1)
    hbm = pl.BlockSpec(memory_space=pl.ANY)
    out = pl.pallas_call(
        _kernel,
        in_specs=[hbm] * 13,
        out_specs=hbm,
        out_shape=jax.ShapeDtypeStruct((rows, D), F32),
        scratch_shapes=[
            pltpu.VMEM((rows, D), BF16),
            pltpu.VMEM((2, P, D), BF16),
            pltpu.VMEM((D, P), BF16),
            pltpu.VMEM((D, P), BF16),
            pltpu.VMEM((D, DF), BF16),
            pltpu.VMEM((D, DF), BF16),
            pltpu.VMEM((DF, D), BF16),
            pltpu.VMEM((2, rows, P), F32),
            pltpu.VMEM((TM, DF), BF16),
            pltpu.VMEM((TM, P), BF16),
            pltpu.VMEM((TM, P), BF16),
            pltpu.VMEM((rows, D), F32),
            pltpu.VMEM((5, 8, P // 8), BF16),
            pltpu.VMEM((10, 8, P), F32),
            pltpu.VMEM((2, 8, D), F32),
            pltpu.VMEM((2, 8, P), F32),
            pltpu.VMEM((8, 128), I32),
            pltpu.SemaphoreType.DMA((rows // TM + 2 * (P // BC) + 2,)),
            pltpu.SemaphoreType.DMA((1,)),
        ],
        compiler_params=pltpu.CompilerParams(vmem_limit_bytes=100 * 1024 * 1024),
    )(A_x.reshape(rows, D), vec(A_Lambda_re), vec(A_Lambda_im), vec(A_log_dt), vec(A_Dskip),
      vec(gate_w), A_B_re, A_B_im, A_C_re, A_C_im, B_w_gate, B_w_up, B_w_down)
    return out.reshape(Bsz, S, D)
```

```python
import math

import jax
import jax.numpy as jnp
from jax import lax
from jax.experimental import pallas as pl
from jax.experimental.pallas import tpu as pltpu

TM = 256
FC = 256
BC = 256
CUTS = (512, 768, 896)

F32 = jnp.float32
BF16 = jnp.bfloat16
I32 = jnp.int32
U32 = jnp.uint32
NT = (((1,), (1,)), ((), ()))
K0 = math.sqrt(2.0 / math.pi)


def _pack(v):
    return pltpu.bitcast(v.astype(BF16), U32)


def _unpack(v):
    return pltpu.bitcast(v, BF16)


def _cmul(ar, ai, br, bi):
    return ar * br - ai * bi, ar * bi + ai * br


def _row(v):
    return jnp.concatenate([v[j:j + 1, :] for j in range(v.shape[0])], axis=1)


def _widen(v, n):
    return v if n == 128 else jnp.concatenate([v] * (n // 128), axis=1)


def _kernel(x_hbm, lre_hbm, lim_hbm, ldt_hbm, dsk_hbm, gw_hbm,
            bre_hbm, bim_hbm, cre_hbm, cim_hbm, wg_hbm, wu_hbm, wd_hbm,
            o_hbm,
            x_v, b_v, cre_v, cim_v, wg_v, wu_v, wd_v,
            u_v, h_v, hr_v, hi_v, o_v, small_v, coef_ref, rows_ref, carry_ref, zero_ref,
            isem, osem):
    tm, fc = TM, FC
    S, D = x_v.shape
    P = b_v.shape[1]
    DF = wg_v.shape[1]
    nR = S // tm
    nB = P // BC

    def x_copy(r):
        rows = pl.ds(r * tm if isinstance(r, int) else pl.multiple_of(r * tm, tm), tm)
        return pltpu.make_async_copy(x_hbm.at[rows, :], x_v.at[rows, :], isem.at[r])

    b_copies = []
    for part, src in enumerate((bre_hbm, bim_hbm)):
        for i in range(nB):
            rows = pl.ds(i * BC, BC)
            b_copies.append(pltpu.make_async_copy(
                src.at[rows, :], b_v.at[part, rows, :], isem.at[nR + part * nB + i]))
    s_copies = [pltpu.make_async_copy(s, small_v.at[i], isem.at[nR + 2 * nB])
                for i, s in enumerate((lre_hbm, lim_hbm, ldt_hbm, dsk_hbm, gw_hbm))]
    w_copies = [pltpu.make_async_copy(s, d, isem.at[nR + 2 * nB + 1])
                for s, d in ((wg_hbm, wg_v), (wu_hbm, wu_v), (wd_hbm, wd_v),
                             (cre_hbm, cre_v), (cim_hbm, cim_v))]

    for c in s_copies:
        c.start()
    x_copy(0).start()
    for c in b_copies:
        c.start()
    for r in range(1, nR):
        x_copy(r).start()
    for c in w_copies:
        c.start()

    for c in s_copies:
        c.wait()
    lre = _row(small_v[0].astype(F32))
    lim = _row(small_v[1].astype(F32))
    dt = jnp.exp(_row(small_v[2].astype(F32))).astype(BF16).astype(F32)
    rows_ref[0] = jnp.broadcast_to(_row(small_v[3].astype(F32)), (8, D))
    rows_ref[1] = jnp.broadcast_to(_row(small_v[4].astype(F32)), (8, D))
    zr = dt * lre
    zi = dt * lim
    sub = lax.broadcasted_iota(I32, (8, P), 0)
    k = jnp.where(sub == 0, 1, jnp.where(sub == 1, 2, 4)).astype(F32)
    mag = jnp.exp(k * zr)
    pwr = mag * jnp.cos(k * zi)
    pwi = mag * jnp.sin(k * zi)
    ar = pwr[0:1] - 1.0
    ai = pwi[0:1]
    den = lre * lre + lim * lim
    coef_ref[0] = jnp.broadcast_to(2.0 * (ar * lre + ai * lim) / den, (8, P))
    coef_ref[1] = jnp.broadcast_to(2.0 * (ai * lre - ar * lim) / den, (8, P))
    coef_ref[2] = jnp.where(sub == 0, jnp.broadcast_to(pwr[0:1], (8, P)), 0.0)
    coef_ref[3] = jnp.where(sub == 0, jnp.broadcast_to(pwi[0:1], (8, P)), 0.0)
    for n, s in enumerate((1, 2, 4)):
        coef_ref[4 + 2 * n] = jnp.where(sub >= s, jnp.broadcast_to(pwr[n:n + 1], (8, P)), 0.0)
        coef_ref[5 + 2 * n] = jnp.where(sub >= s, jnp.broadcast_to(pwi[n:n + 1], (8, P)), 0.0)
    carry_ref[...] = jnp.zeros_like(carry_ref)
    zero_ref[...] = jnp.zeros_like(zero_ref)

    x_copy(0).wait()
    x0 = x_v[0:tm, :]
    for part in range(2):
        for i in range(nB):
            b_copies[part * nB + i].wait()
            u_v[part, 0:tm, i * BC:(i + 1) * BC] = lax.dot_general(
                x0, b_v[part, i * BC:(i + 1) * BC, :], NT, preferred_element_type=F32)

    def phase_a(r, _):
        x_copy(r).wait()
        rows = pl.ds(pl.multiple_of(r * tm, tm), tm)
        x = x_v[rows, :]
        u_v[0, rows, :] = lax.dot_general(x, b_v[0], NT, preferred_element_type=F32)
        u_v[1, rows, :] = lax.dot_general(x, b_v[1], NT, preferred_element_type=F32)
        return 0

    lax.fori_loop(1, nR, phase_a, 0)
    for c in w_copies:
        c.wait()

    cuts = [0, *CUTS, D]

    def o_copy(r, n):
        rows = pl.ds(r * tm if isinstance(r, int) else pl.multiple_of(r * tm, tm), tm)
        cols = pl.ds(cuts[n], cuts[n + 1] - cuts[n])
        return pltpu.make_async_copy(o_v.at[rows, cols], o_hbm.at[rows, cols], osem.at[0])

    def body(r, _):
        r0 = pl.multiple_of(r * tm, tm)
        rows = pl.ds(r0, tm)
        x = x_v[rows, :]
        xf = x.astype(F32)
        logit = jnp.sum(xf * rows_ref[1, 0:1, :], axis=-1, keepdims=True)
        gate = jnp.broadcast_to(jax.nn.sigmoid(logit), (tm, 128))
        ngate = -gate
        rest = 1.0 - gate

        zero = zero_ref[...]
        prev = None
        for j in range(P // 128):
            ln = slice(j * 128, (j + 1) * 128)
            cr, ci = coef_ref[0, :, ln], coef_ref[1, :, ln]
            l0r, l0i = coef_ref[2, :, ln], coef_ref[3, :, ln]
            steps = [(coef_ref[4 + 2 * n, :, ln], coef_ref[5 + 2 * n, :, ln]) for n in range(3)]
            Hr, Hi = carry_ref[0, :, ln], carry_ref[1, :, ln]
            if prev is not None:
                Hr = pltpu.bitcast(pltpu.bitcast(Hr, I32) | (pltpu.bitcast(prev, I32) & zero), F32)
            for q in range(tm // 16):
                outr, outi = [], []
                for t in range(2):
                    k8 = q * 16 + t * 8
                    vr, vi = _cmul(cr, ci, u_v[0, pl.ds(r0 + k8, 8), ln], u_v[1, pl.ds(r0 + k8, 8), ln])
                    vr, vi = vr + (l0r * Hr - l0i * Hi), vi + (l0r * Hi + l0i * Hr)
                    for s, (mr, mi) in zip((1, 2, 4), steps):
                        sr = pltpu.roll(vr, s, 0)
                        si = pltpu.roll(vi, s, 0)
                        vr, vi = vr + (mr * sr - mi * si), vi + (mr * si + mi * sr)
                    Hr = jnp.broadcast_to(vr[7:8], (8, 128))
                    Hi = jnp.broadcast_to(vi[7:8], (8, 128))
                    outr.append(vr * gate[k8:k8 + 8])
                    outi.append(vi * ngate[k8:k8 + 8])
                hr_v[q * 8:q * 8 + 8, ln] = _pack(jnp.concatenate(outr, axis=0))
                hi_v[q * 8:q * 8 + 8, ln] = _pack(jnp.concatenate(outi, axis=0))
            carry_ref[0, :, ln] = Hr
            carry_ref[1, :, ln] = Hi
            prev = Hr

        for c in range(DF // fc):
            cols = slice(c * fc, (c + 1) * fc)
            g = jnp.dot(x, wg_v[:, cols], preferred_element_type=F32)
            u = jnp.dot(x, wu_v[:, cols], preferred_element_type=F32)
            inner = g * (K0 + (K0 * 0.044715) * (g * g))
            h_v[:, cols] = _pack((g * (0.5 + 0.5 * jnp.tanh(inner))) * (u * _widen(rest, fc)))

        acc = (xf * rows_ref[0, 0:1, :]) * _widen(gate, D)
        acc = acc + jnp.dot(_unpack(h_v[...]), wd_v[...], preferred_element_type=F32)
        acc = acc + lax.dot_general(_unpack(hr_v[...]), cre_v[...], NT, preferred_element_type=F32)
        for n, (c0, c1) in enumerate(zip(cuts[:-1], cuts[1:])):
            o_v[rows, c0:c1] = acc[:, c0:c1] + lax.dot_general(
                _unpack(hi_v[...]), cim_v[c0:c1, :], NT, preferred_element_type=F32)
            o_copy(r, n).start()
        return 0

    lax.fori_loop(0, nR, body, 0)
    for r in range(nR):
        for n in range(len(cuts) - 1):
            o_copy(r, n).wait()


@jax.jit
def pallas_gated_mix__ssm_conv_s5__glu_gated_geglu__prompt_kernel(
    A_x: jax.Array,
    A_Lambda_re: jax.Array,
    A_Lambda_im: jax.Array,
    A_B_re: jax.Array,
    A_B_im: jax.Array,
    A_C_re: jax.Array,
    A_C_im: jax.Array,
    A_log_dt: jax.Array,
    A_Dskip: jax.Array,
    B_x: jax.Array,
    B_w_gate: jax.Array,
    B_w_up: jax.Array,
    B_w_down: jax.Array,
    gate_w: jax.Array,
):
    del B_x
    Bsz, S, D = A_x.shape
    P = A_Lambda_re.shape[0]
    DF = B_w_gate.shape[1]
    assert Bsz == 1, "the state is carried across all rows, so there must be one sequence"
    rows = S
    vec = lambda a: a.reshape(8, -1)
    hbm = pl.BlockSpec(memory_space=pl.ANY)
    out = pl.pallas_call(
        _kernel,
        in_specs=[hbm] * 13,
        out_specs=hbm,
        out_shape=jax.ShapeDtypeStruct((rows, D), F32),
        scratch_shapes=[
            pltpu.VMEM((rows, D), BF16),
            pltpu.VMEM((2, P, D), BF16),
            pltpu.VMEM((D, P), BF16),
            pltpu.VMEM((D, P), BF16),
            pltpu.VMEM((D, DF), BF16),
            pltpu.VMEM((D, DF), BF16),
            pltpu.VMEM((DF, D), BF16),
            pltpu.VMEM((2, rows, P), F32),
            pltpu.VMEM((TM // 2, DF), U32),
            pltpu.VMEM((TM // 2, P), U32),
            pltpu.VMEM((TM // 2, P), U32),
            pltpu.VMEM((rows, D), F32),
            pltpu.VMEM((5, 8, P // 8), BF16),
            pltpu.VMEM((10, 8, P), F32),
            pltpu.VMEM((2, 8, D), F32),
            pltpu.VMEM((2, 8, P), F32),
            pltpu.VMEM((8, 128), I32),
            pltpu.SemaphoreType.DMA((rows // TM + 2 * (P // BC) + 2,)),
            pltpu.SemaphoreType.DMA((1,)),
        ],
        compiler_params=pltpu.CompilerParams(vmem_limit_bytes=100 * 1024 * 1024),
    )(A_x.reshape(rows, D), vec(A_Lambda_re), vec(A_Lambda_im), vec(A_log_dt), vec(A_Dskip),
      vec(gate_w), A_B_re, A_B_im, A_C_re, A_C_im, B_w_gate, B_w_up, B_w_down)
    return out.reshape(Bsz, S, D)
```
